```python
import jax
import jax.numpy as jnp

def _softmax(x, axis=-1):
    return jax.nn.softmax(x, axis=axis)
def _gelu(x):
    return jax.nn.gelu(x, approximate=True)
def _silu(x):
    return jax.nn.silu(x)
def _sigmoid(x):
    return jax.nn.sigmoid(x)
def _layernorm(x, axis=-1, eps=1e-5):
    m = jnp.mean(x, axis=axis, keepdims=True)
    v = jnp.var(x, axis=axis, keepdims=True)
    return (x - m) / jnp.sqrt(v + eps)
def _scatter_add(tgt, idx, src, axis=0):
    return tgt.at[idx].add(src)
def _segment_sum(src, seg, n):
    return jax.ops.segment_sum(src, seg, n)
class _Rng:
    def __init__(self, key):
        self._k = key
    def _next(self):
        self._k, sub = jax.random.split(self._k)
        return sub
    def normal(self, shape):
        return jax.random.normal(self._next(), shape, dtype=jnp.bfloat16)
    def randint(self, lo, hi, shape):
        return jax.random.randint(self._next(), shape, lo, hi, dtype=jnp.int32)
    def uniform(self, shape, lo=0.0, hi=1.0):
        return jax.random.uniform(self._next(), shape, jnp.bfloat16, lo, hi)
    def permutation(self, n):
        return jax.random.permutation(self._next(), n)


kernel_name = 'sequential_preLN__mha_block_cached__moe_arch_mod__decode'

def setup_inputs():
    _rng = _Rng(jax.random.key(int.from_bytes(__import__("os").urandom(4), "little")))
    _w = (lambda a: (lambda t: t.astype(jnp.bfloat16) if jnp.issubdtype(t.dtype, jnp.floating) else t)(jnp.asarray(a)))
    def _A_setup():
        B, Sq, D = 4, 1, 640
        H, Sk, Dh = 32, 8192, 192
        return {
            "x": _w((lambda *s: _rng.normal(s) * 0.05)(B, Sq, D)),
            "k_cache": _w((lambda *s: _rng.normal(s) * 0.05)(B, H, Sk, Dh)),
            "v_cache": _w((lambda *s: _rng.normal(s) * 0.05)(B, H, Sk, Dh)),
            "wq": _w((lambda *s: _rng.normal(s) * 0.05)(D, H * Dh) * (D ** -0.5)),
            "wo": _w((lambda *s: _rng.normal(s) * 0.05)(H * Dh, D) * ((H * Dh) ** -0.5)),
        }
    _A_in = _A_setup()

    def _B_setup():
        B, S, D, F, C = 4, 1, 640, 1536, 1
        return {
            "x": _w((lambda *s: _rng.normal(s) * 0.05)(B, S, D)),
            "w_r": _w((lambda *s: _rng.normal(s) * 0.05)(D)),
            "w_gate": _w((lambda *s: _rng.normal(s) * 0.05)(D, F)),
            "w_up": _w((lambda *s: _rng.normal(s) * 0.05)(D, F)),
            "w_down": _w((lambda *s: _rng.normal(s) * 0.05)(F, D)),
        }
    _B_in = _B_setup()

    return {
        "A_x": _A_in["x"],
        "A_k_cache": _A_in["k_cache"],
        "A_v_cache": _A_in["v_cache"],
        "A_wq": _A_in["wq"],
        "A_wo": _A_in["wo"],
        "B_x": _B_in["x"],
        "B_w_r": _B_in["w_r"],
        "B_w_gate": _B_in["w_gate"],
        "B_w_up": _B_in["w_up"],
        "B_w_down": _B_in["w_down"],
    }

def reference(A_x, A_k_cache, A_v_cache, A_wq, A_wo, B_x, B_w_r, B_w_gate, B_w_up, B_w_down):
    def _A_ref(x, k_cache, v_cache, wq, wo):
        B, Sq, D = x.shape
        H, Dh = 32, 192
        q = (lambda x, *d: x.transpose(*d))((x @ wq).reshape(B, Sq, H, Dh), 0, 2, 1, 3)
        scores = jnp.einsum("bhqd,bhkd->bhqk", q, k_cache) * (Dh ** -0.5)
        p = _softmax(scores, axis=-1)
        o = jnp.einsum("bhqk,bhkd->bhqd", p, v_cache)
        return (lambda x, *d: x.transpose(*d))(o, 0, 2, 1, 3).reshape(B, Sq, H * Dh) @ wo

    def _B_ref(x, w_r, w_gate, w_up, w_down):
        B, S, D = x.shape
        C = 1
        r = x @ w_r
        idx = jnp.argsort(-r, axis=-1)[:, :C]
        idx_e = jnp.repeat(idx.reshape(B, C, 1), D, axis=2)
        x_sel = jnp.take_along_axis(x, idx_e, axis=1)
        g = _silu(x_sel @ w_gate)
        u = x_sel @ w_up
        y = (g * u) @ w_down
        r_sel = _sigmoid(jnp.take_along_axis(r, idx, axis=1))
        y = y * r_sel.reshape(B, C, 1)
        b_off = (jnp.arange(B) * S).reshape(B, 1)
        flat_idx = (idx + b_off).reshape(B * C)
        zero = (x * 0.0).reshape(B * S, D)
        upd = _scatter_add(zero, flat_idx, y.reshape(B * C, D), axis=0)
        return x + upd.reshape(B, S, D)

    x = A_x
    h = x + _A_ref(_layernorm(x, axis=-1), A_k_cache, A_v_cache, A_wq, A_wo)
    h2 = h + _B_ref(_layernorm(h, axis=-1), B_w_r, B_w_gate, B_w_up, B_w_down)
    return h2
```

```python
import functools
import jax
import jax.numpy as jnp
from jax.experimental import pallas as pl
from jax.experimental.pallas import tpu as pltpu

B, D_MODEL, H, SK, DH, FF = 4, 640, 32, 8192, 192, 1536
PR = 2 * DH
NG = H // 2
NU = B * NG
EPS = 1e-5
SCALE = DH ** -0.5
F32 = jnp.float32
BF16 = jnp.bfloat16


def _ln(x):
    m = jnp.mean(x, axis=-1, keepdims=True)
    xc = x - m
    v = jnp.mean(xc * xc, axis=-1, keepdims=True)
    return xc * jax.lax.rsqrt(v + EPS)


def _make_kernel(CW=128, RD=64, PK=0, PV=1):
    NC = SK // CW
    TOT = NU * NC

    def kernel(x_hbm, k_hbm, v_hbm, wq_hbm, wo_hbm, wr_hbm, wg_hbm, wu_hbm, wd_hbm, out_ref,
               xbuf, wrbuf, wqbuf, wobuf, wgbuf, wubuf, wdbuf, kbuf, vbuf, s_scr, q_scr, acc_scr,
               ksem, vsem, wsem):

        def unit_row(t):
            g = t // B
            b = t % B
            return pl.multiple_of(b * (H * DH) + g * PR, PR), b, g

        def chunk_src(ref, c):
            t = c // NC
            j = c % NC
            row, _, _ = unit_row(t)
            return ref.at[pl.ds(row, PR), pl.ds(pl.multiple_of(j * CW, CW), CW)]

        def kstart(c, slot):
            pltpu.make_async_copy(chunk_src(k_hbm, c), kbuf.at[slot], ksem.at[slot]).start(priority=PK)

        def vstart(c, slot):
            pltpu.make_async_copy(chunk_src(v_hbm, c), vbuf.at[slot], vsem.at[slot]).start(priority=PV)

        def kwait(slot):
            pltpu.make_async_copy(k_hbm.at[pl.ds(0, PR), pl.ds(0, CW)], kbuf.at[slot], ksem.at[slot]).wait()

        def vwait(slot):
            pltpu.make_async_copy(v_hbm.at[pl.ds(0, PR), pl.ds(0, CW)], vbuf.at[slot], vsem.at[slot]).wait()

        cx = pltpu.make_async_copy(x_hbm, xbuf, wsem.at[0])
        cwq = pltpu.make_async_copy(wq_hbm, wqbuf, wsem.at[1])
        cwo = pltpu.make_async_copy(wo_hbm, wobuf, wsem.at[2])
        cwr = pltpu.make_async_copy(wr_hbm, wrbuf, wsem.at[3])
        cwg = pltpu.make_async_copy(wg_hbm, wgbuf, wsem.at[4])
        cwu = pltpu.make_async_copy(wu_hbm, wubuf, wsem.at[5])
        cwd = pltpu.make_async_copy(wd_hbm, wdbuf, wsem.at[6])

        cx.start(priority=PK)
        cwq.start(priority=PK)
        for c in range(RD):
            kstart(c, c)
        for c in range(RD):
            vstart(c, c)
        cwo.start(priority=PV)
        cwr.start(priority=PV)

        cx.wait()
        x = xbuf[...].astype(F32)
        ln1 = _ln(x).astype(BF16)
        cwq.wait()
        q = jnp.dot(ln1, wqbuf[...], preferred_element_type=F32)
        q_scr[...] = q.astype(BF16).astype(F32)
        acc_scr[...] = jnp.zeros_like(acc_scr)

        row8 = jax.lax.broadcasted_iota(jnp.int32, (8, PR), 0)
        lane8 = jax.lax.broadcasted_iota(jnp.int32, (8, PR), 1)
        bd_mask = ((row8 == 0) & (lane8 < DH)) | ((row8 == 1) & (lane8 >= DH))

        def make_qbd(t):
            _, b, g = unit_row(t)
            qrow = q_scr[pl.ds(b, 1), pl.ds(pl.multiple_of(g * PR, 128), PR)]
            return jnp.where(bd_mask, jnp.broadcast_to(qrow, (8, PR)), 0.0).astype(BF16)

        def run_unit(t, do_qk, do_pv, m_prev, k_more, v_more):
            par = t % 2
            qbd = make_qbd(t) if do_qk else None

            def body(j, carry):
                m_run, l_run, o_acc = carry
                c = t * NC + j
                slot = c % RD
                if do_qk:
                    kwait(slot)
                if do_pv:
                    vwait(slot)
                if do_qk:
                    s = jnp.dot(qbd, kbuf[slot], preferred_element_type=F32)
                    s_scr[par, j] = s
                    m_run = jnp.maximum(m_run, s)
                if do_pv:
                    sp = s_scr[1 - par, j]
                    p = jnp.exp((sp - m_prev) * SCALE)
                    l_run = l_run + p
                    o_acc = o_acc + jax.lax.dot_general(
                        p.astype(BF16), vbuf[slot], (((1,), (1,)), ((), ())), preferred_element_type=F32)
                if do_qk:
                    if k_more is True:
                        kstart(c + RD, slot)
                    elif k_more == 'dyn':
                        @pl.when(c + RD < TOT)
                        def _():
                            kstart(c + RD, slot)
                if do_pv:
                    if v_more is True:
                        vstart(c - NC + RD, slot)
                    elif v_more == 'dyn':
                        @pl.when(c - NC + RD < TOT)
                        def _():
                            vstart(c - NC + RD, slot)
                return m_run, l_run, o_acc

            init = (jnp.full((8, CW), -jnp.inf, F32), jnp.zeros((8, CW), F32), jnp.zeros((8, PR), F32))
            m_run, l_run, o_acc = jax.lax.fori_loop(0, NC, body, init)
            if do_pv:
                _, b, g = unit_row(t - 1)
                l = jnp.sum(l_run, axis=1, keepdims=True)
                o = jnp.where(bd_mask, o_acc / l, 0.0).astype(BF16)
                part = jnp.dot(o, wobuf[pl.ds(pl.multiple_of(g * PR, PR), PR), :], preferred_element_type=F32)
                contrib = jnp.sum(part, axis=0, keepdims=True)
                rowa = jax.lax.broadcasted_iota(jnp.int32, acc_scr.shape, 0)
                acc_scr[...] += jnp.where(rowa == b, jnp.broadcast_to(contrib, acc_scr.shape), 0.0)
            if do_qk:
                m_new = jnp.broadcast_to(jnp.max(m_run, axis=1, keepdims=True), (8, CW))
            else:
                m_new = m_prev
            return m_new

        m0 = run_unit(0, True, False, None, True, None)
        cwo.wait()

        def outer(t, m_prev):
            return run_unit(t, True, True, m_prev, True, True)

        m1 = jax.lax.fori_loop(1, NU - 1, outer, m0)
        m2 = run_unit(NU - 1, True, True, m1, 'dyn', True)
        cwg.start(priority=PV)
        cwu.start(priority=PV)
        cwd.start(priority=PV)
        run_unit(NU, False, True, m2, None, 'dyn')

        cwr.wait()
        attn = acc_scr[0:B, :]
        h = x + attn
        ln2 = _ln(h)
        ln2b = ln2.astype(BF16)
        r = jnp.sum(ln2b.astype(F32) * wrbuf[...].astype(F32), axis=1, keepdims=True)
        cwg.wait()
        cwu.wait()
        gt = jnp.dot(ln2b, wgbuf[...], preferred_element_type=F32)
        up = jnp.dot(ln2b, wubuf[...], preferred_element_type=F32)
        act = (gt * jax.nn.sigmoid(gt) * up).astype(BF16)
        cwd.wait()
        y = jnp.dot(act, wdbuf[...], preferred_element_type=F32)
        out = h + (ln2 + y * jax.nn.sigmoid(r))
        out_ref[...] = out.astype(out_ref.dtype)

    def fn(A_x, A_k_cache, A_v_cache, A_wq, A_wo, B_x, B_w_r, B_w_gate, B_w_up, B_w_down):
        kt = jnp.swapaxes(A_k_cache, 2, 3).reshape(B * H * DH, SK)
        vt = jnp.swapaxes(A_v_cache, 2, 3).reshape(B * H * DH, SK)
        x2 = A_x.reshape(B, D_MODEL)
        wr = B_w_r.reshape(1, D_MODEL)
        anyspec = pl.BlockSpec(memory_space=pl.ANY)
        out = pl.pallas_call(
            kernel,
            in_specs=[anyspec] * 9,
            out_specs=pl.BlockSpec(memory_space=pltpu.VMEM),
            out_shape=jax.ShapeDtypeStruct((B, D_MODEL), BF16),
            scratch_shapes=[
                pltpu.VMEM((B, D_MODEL), BF16),
                pltpu.VMEM((1, D_MODEL), BF16),
                pltpu.VMEM((D_MODEL, H * DH), BF16),
                pltpu.VMEM((H * DH, D_MODEL), BF16),
                pltpu.VMEM((D_MODEL, FF), BF16),
                pltpu.VMEM((D_MODEL, FF), BF16),
                pltpu.VMEM((FF, D_MODEL), BF16),
                pltpu.VMEM((RD, PR, CW), BF16),
                pltpu.VMEM((RD, PR, CW), BF16),
                pltpu.VMEM((2, NC, 8, CW), F32),
                pltpu.VMEM((B, H * DH), F32),
                pltpu.VMEM((8, D_MODEL), F32),
                pltpu.SemaphoreType.DMA((RD,)),
                pltpu.SemaphoreType.DMA((RD,)),
                pltpu.SemaphoreType.DMA((8,)),
            ],
            compiler_params=pltpu.CompilerParams(vmem_limit_bytes=100 * 1024 * 1024),
        )(x2, kt, vt, A_wq, A_wo, wr, B_w_gate, B_w_up, B_w_down)
        return out.reshape(B, 1, D_MODEL)
    return fn


_IMPL = _make_kernel()


@jax.jit
def pallas_sequential_preLN__mha_block_cached__moe_arch_mod__decode_kernel(
    A_x, A_k_cache, A_v_cache, A_wq, A_wo, B_x, B_w_r, B_w_gate, B_w_up, B_w_down
):
    return _IMPL(A_x, A_k_cache, A_v_cache, A_wq, A_wo, B_x, B_w_r, B_w_gate, B_w_up, B_w_down)
```

```python
import jax
import jax.numpy as jnp
from jax import lax
from jax.experimental import pallas as pl
from jax.experimental.pallas import tpu as pltpu

B, D_MODEL, H, SK, DH, FF = 4, 640, 32, 8192, 192, 1536
PR = 2 * DH
NG = H // 2
NU = B * NG
CW = 128
NC = SK // CW
RD = NC // 2
NP = D_MODEL // 128
NGU = NP * (FF // PR)
NWG = FF // PR
EPS = 1e-5
SCALE = DH ** -0.5
F32 = jnp.float32
BF16 = jnp.bfloat16
TA, TB = 0, 1


def _ln(x):
    m = jnp.mean(x, axis=-1, keepdims=True)
    xc = x - m
    v = jnp.mean(xc * xc, axis=-1, keepdims=True)
    return xc * lax.rsqrt(v + EPS)


def _kernel(x_hbm, k_hbm, v_hbm, wq_hbm, wo_hbm, wr_hbm, wg_hbm, wu_hbm, wd_hbm, out_ref,
            xbuf, wrbuf, ln1_scr, wqbuf, wobuf, wgbuf, wubuf, wdbuf, kbuf, vbuf, s_scr, q_scr, acc_scr,
            ksem, vsem, wsem, wqsem, wosem, wdsem):

    def unit_row(t):
        g = lax.shift_right_logical(t, 2)
        b = jnp.bitwise_and(t, B - 1)
        return b * (H * DH) + g * PR

    def chunk_copy(hbm, buf, sem, row, j):
        slot = jnp.bitwise_and(j, RD - 1)
        src = hbm.at[pl.ds(pl.multiple_of(row, PR), PR), pl.ds(pl.multiple_of(j * CW, CW), CW)]
        return pltpu.make_async_copy(src, buf.at[slot], sem.at[slot])

    def kstart(row, j, prio):
        chunk_copy(k_hbm, kbuf, ksem, row, j).start(priority=prio)

    def vstart(row, j, prio):
        chunk_copy(v_hbm, vbuf, vsem, row, j).start(priority=prio)

    def wq_copy(g, p):
        par = jnp.bitwise_and(g, 1)
        rows = pl.ds(pl.multiple_of(p * 128, 128), 128)
        return pltpu.make_async_copy(
            wq_hbm.at[rows, pl.ds(pl.multiple_of(g * PR, 128), PR)], wqbuf.at[par, rows], wqsem.at[par])

    def wo_copy(g, p):
        par = jnp.bitwise_and(g, 1)
        cols = pl.ds(pl.multiple_of(p * 128, 128), 128)
        return pltpu.make_async_copy(
            wo_hbm.at[pl.ds(pl.multiple_of(g * PR, PR), PR), cols], wobuf.at[par, :, cols], wosem.at[par])

    def gu_copy(hbm, buf, sem, cg, p):
        sl = (pl.ds(pl.multiple_of(p * 128, 128), 128), pl.ds(pl.multiple_of(cg * PR, 128), PR))
        return pltpu.make_async_copy(hbm.at[sl], buf.at[sl], sem)

    def wd_copy(rg, p):
        sl = (pl.ds(pl.multiple_of(rg * PR, PR), PR), pl.ds(pl.multiple_of(p * 128, 128), 128))
        return pltpu.make_async_copy(wd_hbm.at[sl], wdbuf.at[sl], wdsem.at[rg])

    cx = pltpu.make_async_copy(x_hbm, xbuf, wsem.at[0])
    cwr = pltpu.make_async_copy(wr_hbm, wrbuf, wsem.at[1])

    cx.start(priority=TB)

    def first_weights(p, c):
        wq_copy(0, p).start(priority=TA)
        wo_copy(0, p).start(priority=TB)
        return c
    lax.fori_loop(0, NP, first_weights, 0)

    row0 = unit_row(0)

    def fill(i, c):
        kstart(row0, 2 * i, TA)
        kstart(row0, 2 * i + 1, TB)
        return c
    lax.fori_loop(0, RD // 2, fill, 0)
    wq_copy(1, 0).start(priority=TA)
    cwr.start(priority=TB)
    wq_copy(1, NP - 1).start(priority=TA)

    cx.wait()
    ln1_scr[...] = _ln(xbuf[...].astype(F32)).astype(BF16)
    acc_scr[...] = jnp.zeros_like(acc_scr)

    row8 = lax.broadcasted_iota(jnp.int32, (8, PR), 0)
    lane8 = lax.broadcasted_iota(jnp.int32, (8, PR), 1)
    bd_mask = ((row8 == 0) & (lane8 < DH)) | ((row8 == 1) & (lane8 >= DH))

    def issue_ffn():
        def gate_up(cg, c):
            def piece(p, c2):
                gu_copy(wg_hbm, wgbuf, wsem.at[2], cg, p).start(priority=TA)
                gu_copy(wu_hbm, wubuf, wsem.at[3], cg, p).start(priority=TB)
                return c2
            return lax.fori_loop(0, NP, piece, c)
        lax.fori_loop(0, FF // PR, gate_up, 0)

        def down_lo(p, c):
            wd_copy(0, p).start(priority=TA)
            wd_copy(1, p).start(priority=TB)
            return c
        lax.fori_loop(0, NP, down_lo, 0)

        def down_hi(p, c):
            wd_copy(2, p).start(priority=TA)
            wd_copy(3, p).start(priority=TB)
            return c
        lax.fori_loop(0, NP, down_hi, 0)

    def chunk_loop(t, do_qk, do_pv, m_prev, kmode, vmode, unroll, lo, hi, carry):
        par = jnp.bitwise_and(t, 1)
        if do_qk:
            qrow = q_scr[pl.ds(jnp.bitwise_and(t, B - 1), 1), :]
            qbd = jnp.where(bd_mask, jnp.broadcast_to(qrow, (8, PR)), 0.0).astype(BF16)

        def body(jj, carry):
            m_run, l_run, o_acc = carry
            js = [jj * unroll + u for u in range(unroll)]
            slots = [jnp.bitwise_and(j, RD - 1) for j in js]
            for j in js:
                if do_qk:
                    chunk_copy(k_hbm, kbuf, ksem, 0, j).wait()
                if do_pv:
                    chunk_copy(v_hbm, vbuf, vsem, 0, j).wait()
            if do_pv:
                for j, slot in zip(js, slots):
                    p = jnp.exp((s_scr[1 - par, j] - m_prev) * SCALE)
                    l_run = l_run + p
                    o_acc = o_acc + lax.dot_general(
                        p.astype(BF16), vbuf[slot], (((1,), (1,)), ((), ())), preferred_element_type=F32)
            if do_qk:
                for j, slot in zip(js, slots):
                    s = jnp.dot(qbd, kbuf[slot], preferred_element_type=F32)
                    s_scr[par, j] = s
                    m_run = jnp.maximum(m_run, s)
            for u in range(unroll):
                for start, mode in ((kstart, kmode), (vstart, vmode)):
                    if mode is None:
                        continue
                    if len(mode) == 3:
                        start(mode[0], js[u] + mode[1], mode[2][u])
                    else:
                        jn = js[u] + RD
                        start(jnp.where(jn < NC, mode[0], mode[1]), jnp.bitwise_and(jn, NC - 1), mode[2][u])
            return m_run, l_run, o_acc

        return lax.fori_loop(lo // unroll, hi // unroll, body, carry)

    def run_unit(t, m_prev, kind):
        r_prev, r_cur, r_next = unit_row(t - 1), unit_row(t), unit_row(t + 1)
        carry = (jnp.full((8, CW), -jnp.inf, F32), jnp.zeros((8, CW), F32), jnp.zeros((8, PR), F32))
        do_qk = kind != 'last_pv'
        do_pv = kind != 'first'
        if kind == 'first':
            carry = chunk_loop(t, True, False, m_prev, (r_cur, RD, [TA]), (r_cur, 0, [TB]), 1, 0, RD, carry)
            carry = chunk_loop(t, True, False, m_prev, (r_next, -RD, [TA, TB]), None, 2, RD, NC, carry)
        elif kind == 'mid':
            carry = chunk_loop(t, True, True, m_prev, (r_cur, r_next, [TA], None), (r_prev, r_cur, [TB], None),
                               1, 0, NC, carry)
        elif kind == 'last_qk':
            carry = chunk_loop(t, True, True, m_prev, (r_cur, RD, [TA]), (r_prev, RD, [TB]), 1, 0, RD, carry)
            carry = chunk_loop(t, True, True, m_prev, None, (r_cur, -RD, [TA, TB]), 2, RD, NC, carry)
        else:
            carry = chunk_loop(t, False, True, m_prev, None, (r_prev, RD, [TA, TB]), 2, 0, RD, carry)
            issue_ffn()
            carry = chunk_loop(t, False, True, m_prev, None, None, 2, RD, NC, carry)
        m_run, l_run, o_acc = carry
        if do_pv:
            b = jnp.bitwise_and(t - 1, B - 1)
            g = lax.shift_right_logical(t - 1, 2)

            @pl.when(b == 0)
            def _():
                for p in range(NP):
                    wo_copy(g, p).wait()
            l = jnp.sum(l_run, axis=1, keepdims=True)
            o = jnp.where(bd_mask, o_acc / l, 0.0).astype(BF16)
            part = jnp.dot(o, wobuf[jnp.bitwise_and(g, 1)], preferred_element_type=F32)
            contrib = jnp.sum(part, axis=0, keepdims=True)
            rowa = lax.broadcasted_iota(jnp.int32, acc_scr.shape, 0)
            acc_scr[...] += jnp.where(rowa == b, jnp.broadcast_to(contrib, acc_scr.shape), 0.0)
        if do_qk:
            return jnp.broadcast_to(jnp.max(m_run, axis=1, keepdims=True), (8, CW))
        return m_prev

    def unit_head(t):
        g = lax.shift_right_logical(t, 2)

        @pl.when(jnp.bitwise_and(t, B - 1) == 0)
        def _():
            for p in range(NP):
                wq_copy(g, p).wait()
            q = jnp.dot(ln1_scr[...], wqbuf[jnp.bitwise_and(g, 1)], preferred_element_type=F32)
            q_scr[...] = q.astype(BF16).astype(F32)

    def unit_tail(t):
        g = lax.shift_right_logical(t, 2)
        b = jnp.bitwise_and(t, B - 1)
        g1 = lax.shift_right_logical(t + 1, 2)
        b1 = jnp.bitwise_and(t + 1, B - 1)

        @pl.when(g1 + 1 < NG)
        def _():
            wq_copy(g1 + 1, b1).start(priority=TA)

        @pl.when(g + 1 < NG)
        def _():
            wo_copy(g + 1, b).start(priority=TB)

        @pl.when((b1 == 0) & (g1 + 1 < NG))
        def _():
            wq_copy(g1 + 1, NP - 1).start(priority=TA)

        @pl.when((b == B - 1) & (g + 1 < NG))
        def _():
            wo_copy(g + 1, NP - 1).start(priority=TB)

    unit_head(0)
    m0 = run_unit(0, None, 'first')
    unit_tail(0)

    def outer(t, m_prev):
        unit_head(t)
        m = run_unit(t, m_prev, 'mid')
        unit_tail(t)
        return m

    m1 = lax.fori_loop(1, NU - 1, outer, m0)
    m2 = run_unit(NU - 1, m1, 'last_qk')
    run_unit(NU, m2, 'last_pv')

    cwr.wait()
    h = xbuf[...].astype(F32) + acc_scr[0:B, :]
    ln2 = _ln(h)
    ln2b = ln2.astype(BF16)
    r = jnp.sum(ln2b.astype(F32) * wrbuf[...].astype(F32)[None, :], axis=1, keepdims=True)
    pltpu.make_async_copy(wg_hbm, wgbuf, wsem.at[2]).wait()
    pltpu.make_async_copy(wu_hbm, wubuf, wsem.at[3]).wait()
    gt = jnp.dot(ln2b, wgbuf[...], preferred_element_type=F32)
    up = jnp.dot(ln2b, wubuf[...], preferred_element_type=F32)
    act = (gt * jax.nn.sigmoid(gt) * up).astype(BF16)
    y = jnp.zeros((B, D_MODEL), F32)
    for i in range(NWG):
        sl = pl.ds(i * PR, PR)
        pltpu.make_async_copy(wd_hbm.at[sl], wdbuf.at[sl], wdsem.at[i]).wait()
        y = y + jnp.dot(act[:, i * PR:(i + 1) * PR], wdbuf[sl, :], preferred_element_type=F32)
    out = h + (ln2 + y * jax.nn.sigmoid(r))
    out_ref[...] = out.astype(out_ref.dtype)


@jax.jit
def pallas_sequential_preLN__mha_block_cached__moe_arch_mod__decode_kernel(
    A_x, A_k_cache, A_v_cache, A_wq, A_wo, B_x, B_w_r, B_w_gate, B_w_up, B_w_down
):
    del B_x
    kt = jnp.swapaxes(A_k_cache, 2, 3).reshape(B * H * DH, SK)
    vt = jnp.swapaxes(A_v_cache, 2, 3).reshape(B * H * DH, SK)
    x2 = A_x.reshape(B, D_MODEL)
    anyspec = pl.BlockSpec(memory_space=pl.ANY)
    ring = pltpu.VMEM((RD, PR, CW), BF16)
    out = pl.pallas_call(
        _kernel,
        in_specs=[anyspec] * 9,
        out_specs=pl.BlockSpec(memory_space=pltpu.VMEM),
        out_shape=jax.ShapeDtypeStruct((B, D_MODEL), BF16),
        scratch_shapes=[
            pltpu.VMEM((B, D_MODEL), BF16),
            pltpu.VMEM((D_MODEL,), BF16),
            pltpu.VMEM((B, D_MODEL), BF16),
            pltpu.VMEM((2, D_MODEL, PR), BF16),
            pltpu.VMEM((2, PR, D_MODEL), BF16),
            pltpu.VMEM((D_MODEL, FF), BF16),
            pltpu.VMEM((D_MODEL, FF), BF16),
            pltpu.VMEM((FF, D_MODEL), BF16),
            ring, ring,
            pltpu.VMEM((2, NC, 8, CW), F32),
            pltpu.VMEM((B, PR), F32),
            pltpu.VMEM((8, D_MODEL), F32),
            pltpu.SemaphoreType.DMA((RD,)),
            pltpu.SemaphoreType.DMA((RD,)),
            pltpu.SemaphoreType.DMA((4,)),
            pltpu.SemaphoreType.DMA((2,)),
            pltpu.SemaphoreType.DMA((2,)),
            pltpu.SemaphoreType.DMA((NWG,)),
        ],
        compiler_params=pltpu.CompilerParams(vmem_limit_bytes=64 * 1024 * 1024),
    )(x2, kt, vt, A_wq, A_wo, B_w_r, B_w_gate, B_w_up, B_w_down)
    return out.reshape(B, 1, D_MODEL)
```

```python
import jax
import jax.numpy as jnp
from jax import lax
from jax.experimental import pallas as pl
from jax.experimental.pallas import tpu as pltpu

B, D_MODEL, H, SK, DH, FF = 4, 640, 32, 8192, 192, 1536
PR = 2 * DH
NG = H // 2
NU = B * NG
CW = 128
NC = SK // CW
NP = D_MODEL // 128
NWG = FF // PR
RD = NC // 2
NS = 2
WS = 2
TA, TB = 0, 1
EPS = 1e-5
SCALE = DH ** -0.5
F32 = jnp.float32
BF16 = jnp.bfloat16


def _ln(x):
    m = jnp.mean(x, axis=-1, keepdims=True)
    xc = x - m
    v = jnp.mean(xc * xc, axis=-1, keepdims=True)
    return xc * lax.rsqrt(v + EPS)


def _kernel(x_hbm, k_hbm, v_hbm, wq_hbm, wo_hbm, wr_hbm, wg_hbm, wu_hbm, wd_hbm, out_ref,
            xbuf, wrbuf, ln1_scr, wqbuf, wobuf, wgbuf, wubuf, wdbuf, kbuf, vbuf, s_scr, q_scr, acc_scr,
            ksem, vsem, wsem, wqsem, wosem, wdsem):

    def unit_row(t):
        g = lax.shift_right_logical(t, 2)
        b = jnp.bitwise_and(t, B - 1)
        return b * (H * DH) + g * PR

    def start_pair(a, b, n):
        for i in range(n):
            for (src, dst, sem), prio in ((a, TA), (b, TB)):
                rows = src.shape[0] // n
                sl = pl.ds(i * rows, rows)
                pltpu.make_async_copy(src.at[sl], dst.at[sl], sem).start(priority=prio)

    def wait(d):
        pltpu.make_async_copy(*d).wait()

    def chunk(hbm, buf, sem, row, j):
        slot = jnp.bitwise_and(j, RD - 1)
        src = hbm.at[pl.ds(pl.multiple_of(row, PR), PR), pl.ds(pl.multiple_of(j * CW, CW), CW)]
        return src, buf.at[slot], sem.at[slot]

    def kch(row, j):
        return chunk(k_hbm, kbuf, ksem, row, j)

    def vch(row, j):
        return chunk(v_hbm, vbuf, vsem, row, j)

    def wq_piece(g, p):
        par = jnp.bitwise_and(g, 1)
        rows = pl.ds(pl.multiple_of(p * 128, 128), 128)
        return (wq_hbm.at[rows, pl.ds(pl.multiple_of(g * PR, 128), PR)], wqbuf.at[par, rows], wqsem.at[par])

    def wo_piece(g, p):
        par = jnp.bitwise_and(g, 1)
        cols = pl.ds(pl.multiple_of(p * 128, 128), 128)
        return (wo_hbm.at[pl.ds(pl.multiple_of(g * PR, PR), PR), cols], wobuf.at[par, :, cols], wosem.at[par])

    def gu_piece(hbm, buf, sem, cg, p):
        sl = (pl.ds(pl.multiple_of(p * 128, 128), 128), pl.ds(pl.multiple_of(cg * PR, 128), PR))
        return hbm.at[sl], buf.at[sl], sem

    def wd_piece(rg, p):
        sl = (pl.ds(pl.multiple_of(rg * PR, PR), PR), pl.ds(pl.multiple_of(p * 128, 128), 128))
        return wd_hbm.at[sl], wdbuf.at[sl], wdsem.at[rg]

    cx = pltpu.make_async_copy(x_hbm, xbuf, wsem.at[0])
    cwr = pltpu.make_async_copy(wr_hbm, wrbuf, wsem.at[1])

    cx.start(priority=TB)

    def first_weights(p, c):
        start_pair(wq_piece(0, p), wo_piece(0, p), WS)
        return c
    lax.fori_loop(0, NP, first_weights, 0)

    row0 = unit_row(0)

    def fill(i, c):
        start_pair(kch(row0, 2 * i), kch(row0, 2 * i + 1), NS)
        return c
    lax.fori_loop(0, RD // 2, fill, 0)
    start_pair(wq_piece(1, 0), wq_piece(1, NP - 1), WS)
    cwr.start(priority=TA)

    cx.wait()
    ln1_scr[...] = _ln(xbuf[...].astype(F32)).astype(BF16)
    acc_scr[...] = jnp.zeros_like(acc_scr)

    row8 = lax.broadcasted_iota(jnp.int32, (8, PR), 0)
    lane8 = lax.broadcasted_iota(jnp.int32, (8, PR), 1)
    bd_mask = ((row8 == 0) & (lane8 < DH)) | ((row8 == 1) & (lane8 >= DH))

    def issue_ffn():
        def gate_up(cg, c):
            def piece(p, c2):
                start_pair(gu_piece(wg_hbm, wgbuf, wsem.at[2], cg, p), gu_piece(wu_hbm, wubuf, wsem.at[3], cg, p), WS)
                return c2
            return lax.fori_loop(0, NP, piece, c)
        lax.fori_loop(0, FF // PR, gate_up, 0)

        def down(h2, c):
            def piece(p, c2):
                start_pair(wd_piece(2 * h2, p), wd_piece(2 * h2 + 1, p), WS)
                return c2
            return lax.fori_loop(0, NP, piece, c)
        lax.fori_loop(0, NWG // 2, down, 0)

    def chunk_loop(t, do_qk, do_pv, m_prev, refill, unroll, lo, hi, carry):
        par = jnp.bitwise_and(t, 1)
        if do_qk:
            qrow = q_scr[pl.ds(jnp.bitwise_and(t, B - 1), 1), :]
            qbd = jnp.where(bd_mask, jnp.broadcast_to(qrow, (8, PR)), 0.0).astype(BF16)

        def body(jj, carry):
            m_run, l_run, o_acc = carry
            js = [jj * unroll + u for u in range(unroll)]
            slots = [jnp.bitwise_and(j, RD - 1) for j in js]
            for j in js:
                if do_qk:
                    wait(kch(0, j))
                if do_pv:
                    wait(vch(0, j))
            if do_pv:
                for j, slot in zip(js, slots):
                    p = jnp.exp((s_scr[1 - par, j] - m_prev) * SCALE)
                    l_run = l_run + p
                    o_acc = o_acc + lax.dot_general(
                        p.astype(BF16), vbuf[slot], (((1,), (1,)), ((), ())), preferred_element_type=F32)
            if do_qk:
                for j, slot in zip(js, slots):
                    s = jnp.dot(qbd, kbuf[slot], preferred_element_type=F32)
                    s_scr[par, j] = s
                    m_run = jnp.maximum(m_run, s)
            if refill is not None:
                refill(js)
            return m_run, l_run, o_acc

        return lax.fori_loop(lo // unroll, hi // unroll, body, carry)

    def ahead(make, row_cur, row_next, j):
        jn = j + RD
        return make(jnp.where(jn < NC, row_cur, row_next), jnp.bitwise_and(jn, NC - 1))

    def run_unit(t, m_prev, kind):
        r_prev, r_cur, r_next = unit_row(t - 1), unit_row(t), unit_row(t + 1)
        carry = (jnp.full((8, CW), -jnp.inf, F32), jnp.zeros((8, CW), F32), jnp.zeros((8, PR), F32))
        do_qk = kind != 'last_pv'
        do_pv = kind != 'first'
        both = lambda js: start_pair(ahead(kch, r_cur, r_next, js[0]), ahead(vch, r_prev, r_cur, js[0]), NS)
        if kind == 'first':
            carry = chunk_loop(
                t, True, False, m_prev,
                lambda js: start_pair(ahead(kch, r_cur, r_next, js[0]), vch(r_cur, js[0]), NS), 1, 0, RD, carry)
            carry = chunk_loop(
                t, True, False, m_prev,
                lambda js: start_pair(ahead(kch, r_cur, r_next, js[0]), ahead(kch, r_cur, r_next, js[1]), NS),
                2, RD, NC, carry)
        elif kind == 'mid':
            carry = chunk_loop(t, True, True, m_prev, both, 1, 0, NC, carry)
        elif kind == 'last_qk':
            carry = chunk_loop(
                t, True, True, m_prev,
                lambda js: start_pair(kch(r_cur, js[0] + RD), vch(r_prev, js[0] + RD), NS), 1, 0, NC - RD, carry)
            carry = chunk_loop(
                t, True, True, m_prev,
                lambda js: start_pair(vch(r_cur, js[0] + RD - NC), vch(r_cur, js[1] + RD - NC), NS),
                2, NC - RD, NC, carry)
        else:
            carry = chunk_loop(
                t, False, True, m_prev,
                lambda js: start_pair(vch(r_prev, js[0] + RD), vch(r_prev, js[1] + RD), NS), 2, 0, NC - RD, carry)
            issue_ffn()
            carry = chunk_loop(t, False, True, m_prev, None, 2, NC - RD, NC, carry)
        m_run, l_run, o_acc = carry
        if do_pv:
            b = jnp.bitwise_and(t - 1, B - 1)
            g = lax.shift_right_logical(t - 1, 2)

            @pl.when(b == 0)
            def _():
                for p in range(NP):
                    wait(wo_piece(g, p))
            l = jnp.sum(l_run, axis=1, keepdims=True)
            o = jnp.where(bd_mask, o_acc / l, 0.0).astype(BF16)
            part = jnp.dot(o, wobuf[jnp.bitwise_and(g, 1)], preferred_element_type=F32)
            contrib = jnp.sum(part, axis=0, keepdims=True)
            rowa = lax.broadcasted_iota(jnp.int32, acc_scr.shape, 0)
            acc_scr[...] += jnp.where(rowa == b, jnp.broadcast_to(contrib, acc_scr.shape), 0.0)
        if do_qk:
            return jnp.broadcast_to(jnp.max(m_run, axis=1, keepdims=True), (8, CW))
        return m_prev

    def unit_head(t):
        g = lax.shift_right_logical(t, 2)

        @pl.when(jnp.bitwise_and(t, B - 1) == 0)
        def _():
            for p in range(NP):
                wait(wq_piece(g, p))
            q = jnp.dot(ln1_scr[...], wqbuf[jnp.bitwise_and(g, 1)], preferred_element_type=F32)
            q_scr[...] = q.astype(BF16).astype(F32)

    def unit_tail(t):
        g = lax.shift_right_logical(t, 2)
        b = jnp.bitwise_and(t, B - 1)
        g1 = lax.shift_right_logical(t + 1, 2)
        b1 = jnp.bitwise_and(t + 1, B - 1)

        @pl.when(g1 + 1 < NG)
        def _():
            start_pair(wq_piece(g1 + 1, b1), wo_piece(g + 1, b), WS)

        @pl.when((b == B - 1) & (g1 + 1 < NG))
        def _():
            start_pair(wq_piece(g1 + 1, NP - 1), wo_piece(g + 1, NP - 1), WS)

        @pl.when((b == B - 1) & (g1 + 1 == NG))
        def _():
            start_pair(wo_piece(g + 1, B - 1), wo_piece(g + 1, NP - 1), WS)

    unit_head(0)
    m0 = run_unit(0, None, 'first')
    unit_tail(0)

    def outer(t, m_prev):
        unit_head(t)
        m = run_unit(t, m_prev, 'mid')
        unit_tail(t)
        return m

    m1 = lax.fori_loop(1, NU - 1, outer, m0)
    m2 = run_unit(NU - 1, m1, 'last_qk')
    run_unit(NU, m2, 'last_pv')

    cwr.wait()
    h = xbuf[...].astype(F32) + acc_scr[0:B, :]
    ln2 = _ln(h)
    ln2b = ln2.astype(BF16)
    r = jnp.sum(ln2b.astype(F32) * wrbuf[...].astype(F32)[None, :], axis=1, keepdims=True)
    pltpu.make_async_copy(wg_hbm, wgbuf, wsem.at[2]).wait()
    pltpu.make_async_copy(wu_hbm, wubuf, wsem.at[3]).wait()
    gt = jnp.dot(ln2b, wgbuf[...], preferred_element_type=F32)
    up = jnp.dot(ln2b, wubuf[...], preferred_element_type=F32)
    act = (gt * jax.nn.sigmoid(gt) * up).astype(BF16)
    y = jnp.zeros((B, D_MODEL), F32)
    for i in range(NWG):
        sl = pl.ds(i * PR, PR)
        pltpu.make_async_copy(wd_hbm.at[sl], wdbuf.at[sl], wdsem.at[i]).wait()
        y = y + jnp.dot(act[:, i * PR:(i + 1) * PR], wdbuf[sl, :], preferred_element_type=F32)
    out = h + (ln2 + y * jax.nn.sigmoid(r))
    out_ref[...] = out.astype(out_ref.dtype)


@jax.jit
def pallas_sequential_preLN__mha_block_cached__moe_arch_mod__decode_kernel(
    A_x, A_k_cache, A_v_cache, A_wq, A_wo, B_x, B_w_r, B_w_gate, B_w_up, B_w_down
):
    del B_x
    kt = jnp.swapaxes(A_k_cache, 2, 3).reshape(B * H * DH, SK)
    vt = jnp.swapaxes(A_v_cache, 2, 3).reshape(B * H * DH, SK)
    x2 = A_x.reshape(B, D_MODEL)
    anyspec = pl.BlockSpec(memory_space=pl.ANY)
    ring = pltpu.VMEM((RD, PR, CW), BF16)
    out = pl.pallas_call(
        _kernel,
        in_specs=[anyspec] * 9,
        out_specs=pl.BlockSpec(memory_space=pltpu.VMEM),
        out_shape=jax.ShapeDtypeStruct((B, D_MODEL), BF16),
        scratch_shapes=[
            pltpu.VMEM((B, D_MODEL), BF16),
            pltpu.VMEM((D_MODEL,), BF16),
            pltpu.VMEM((B, D_MODEL), BF16),
            pltpu.VMEM((2, D_MODEL, PR), BF16),
            pltpu.VMEM((2, PR, D_MODEL), BF16),
            pltpu.VMEM((D_MODEL, FF), BF16),
            pltpu.VMEM((D_MODEL, FF), BF16),
            pltpu.VMEM((FF, D_MODEL), BF16),
            ring, ring,
            pltpu.VMEM((2, NC, 8, CW), F32),
            pltpu.VMEM((B, PR), F32),
            pltpu.VMEM((8, D_MODEL), F32),
            pltpu.SemaphoreType.DMA((RD,)),
            pltpu.SemaphoreType.DMA((RD,)),
            pltpu.SemaphoreType.DMA((4,)),
            pltpu.SemaphoreType.DMA((2,)),
            pltpu.SemaphoreType.DMA((2,)),
            pltpu.SemaphoreType.DMA((NWG,)),
        ],
        compiler_params=pltpu.CompilerParams(vmem_limit_bytes=64 * 1024 * 1024),
    )(x2, kt, vt, A_wq, A_wo, B_w_r, B_w_gate, B_w_up, B_w_down)
    return out.reshape(B, 1, D_MODEL)
```

```python
import jax
import jax.numpy as jnp
from jax import lax
from jax.experimental import pallas as pl
from jax.experimental.pallas import tpu as pltpu

B, D_MODEL, H, SK, DH, FF = 4, 640, 32, 8192, 192, 1536
PR = 2 * DH
NG = H // 2
NU = B * NG
CW = 128
NC = SK // CW
NP = D_MODEL // 128
NWG = FF // PR
RD = 16
NS = 4
RT = PR // 8
TA, TB = 0, 1
EPS = 1e-5
SCALE = DH ** -0.5
F32 = jnp.float32
BF16 = jnp.bfloat16


def _ln(x):
    m = jnp.mean(x, axis=-1, keepdims=True)
    xc = x - m
    v = jnp.mean(xc * xc, axis=-1, keepdims=True)
    return xc * lax.rsqrt(v + EPS)


def _kernel(x_hbm, k_hbm, v_hbm, wq_hbm, wo_hbm, wr_hbm, wg_hbm, wu_hbm, wd_hbm, out_ref,
            xbuf, wrbuf, ln1_scr, wqbuf, wobuf, wgbuf, wubuf, wdbuf, kbuf, vbuf, s_scr, q_scr, acc_scr,
            ksem, vsem, wsem, wqsem, wosem, wdsem):

    def unit_row(t):
        g = lax.shift_right_logical(t, 2)
        b = jnp.bitwise_and(t, B - 1)
        return b * (H * DH // 8) + g * RT

    def start_pair(a, b):
        for (src, dst, sem), prio in ((a, TA), (b, TB)):
            pltpu.make_async_copy(src, dst, sem).start(priority=prio)

    def start_chunks(a, b):
        rows = 8 // NS
        for i in range(NS):
            sl = (slice(None), pl.ds(i * rows, rows))
            start_pair((a[0].at[sl], a[1].at[sl], a[2]), (b[0].at[sl], b[1].at[sl], b[2]))

    def wait(d):
        pltpu.make_async_copy(*d).wait()

    def chunk(hbm, buf, sem, row, j):
        slot = jnp.bitwise_and(j, RD - 1)
        src = hbm.at[pl.ds(pl.multiple_of(row, RT), RT), :, pl.ds(pl.multiple_of(j * CW, CW), CW)]
        return src, buf.at[slot], sem.at[slot]

    def kch(row, j):
        return chunk(k_hbm, kbuf, ksem, row, j)

    def vch(row, j):
        return chunk(v_hbm, vbuf, vsem, row, j)

    def wq_piece(g, p):
        par = jnp.bitwise_and(g, 1)
        rows = pl.ds(pl.multiple_of(p * 128, 128), 128)
        return (wq_hbm.at[rows, pl.ds(pl.multiple_of(g * PR, 128), PR)], wqbuf.at[par, rows], wqsem.at[par])

    def wo_piece(g, p):
        par = jnp.bitwise_and(g, 1)
        cols = pl.ds(pl.multiple_of(p * 128, 128), 128)
        return (wo_hbm.at[pl.ds(pl.multiple_of(g * PR, PR), PR), cols], wobuf.at[par, :, cols], wosem.at[par])

    def gu_piece(hbm, buf, sem, cg, p):
        sl = (pl.ds(pl.multiple_of(p * 128, 128), 128), pl.ds(pl.multiple_of(cg * PR, 128), PR))
        return hbm.at[sl], buf.at[sl], sem

    def wd_piece(rg, p):
        sl = (pl.ds(pl.multiple_of(rg * PR, PR), PR), pl.ds(pl.multiple_of(p * 128, 128), 128))
        return wd_hbm.at[sl], wdbuf.at[sl], wdsem.at[rg]

    cx = pltpu.make_async_copy(x_hbm, xbuf, wsem.at[0])
    cwr = pltpu.make_async_copy(wr_hbm, wrbuf, wsem.at[1])

    cx.start(priority=TB)

    def first_weights(p, c):
        start_pair(wq_piece(0, p), wo_piece(0, p))
        return c
    lax.fori_loop(0, NP, first_weights, 0)

    row0 = unit_row(0)

    def fill(i, c):
        start_chunks(kch(row0, 2 * i), kch(row0, 2 * i + 1))
        return c
    lax.fori_loop(0, RD // 2, fill, 0)
    start_pair(wq_piece(1, 0), wq_piece(1, NP - 1))
    cwr.start(priority=TA)

    cx.wait()
    ln1_scr[...] = _ln(xbuf[...].astype(F32)).astype(BF16)
    acc_scr[...] = jnp.zeros_like(acc_scr)

    row8 = lax.broadcasted_iota(jnp.int32, (8, PR), 0)
    lane8 = lax.broadcasted_iota(jnp.int32, (8, PR), 1)
    bd_mask = ((row8 == 0) & (lane8 < DH)) | ((row8 == 1) & (lane8 >= DH))

    def issue_ffn():
        def gate_up(cg, c):
            def piece(p, c2):
                start_pair(gu_piece(wg_hbm, wgbuf, wsem.at[2], cg, p), gu_piece(wu_hbm, wubuf, wsem.at[3], cg, p))
                return c2
            return lax.fori_loop(0, NP, piece, c)
        lax.fori_loop(0, FF // PR, gate_up, 0)

        def down(h2, c):
            def piece(p, c2):
                start_pair(wd_piece(2 * h2, p), wd_piece(2 * h2 + 1, p))
                return c2
            return lax.fori_loop(0, NP, piece, c)
        lax.fori_loop(0, NWG // 2, down, 0)

    def chunk_loop(t, do_qk, do_pv, m_prev, refill, unroll, lo, hi, carry):
        par = jnp.bitwise_and(t, 1)
        if do_qk:
            qrow = q_scr[pl.ds(jnp.bitwise_and(t, B - 1), 1), :]
            qbd = jnp.where(bd_mask, jnp.broadcast_to(qrow, (8, PR)), 0.0).astype(BF16)

        def body(jj, carry):
            m_run, l_run, o_acc = carry
            js = [jj * unroll + u for u in range(unroll)]
            slots = [jnp.bitwise_and(j, RD - 1) for j in js]
            for j in js:
                if do_qk:
                    wait(kch(0, j))
                if do_pv:
                    wait(vch(0, j))
            if do_pv:
                for j, slot in zip(js, slots):
                    p = jnp.exp((s_scr[1 - par, j] - m_prev) * SCALE)
                    l_run = l_run + p
                    o_acc = o_acc + lax.dot_general(
                        p.astype(BF16), vbuf[slot].reshape(PR, CW), (((1,), (1,)), ((), ())),
                        preferred_element_type=F32)
            if do_qk:
                for j, slot in zip(js, slots):
                    s = jnp.dot(qbd, kbuf[slot].reshape(PR, CW), preferred_element_type=F32)
                    s_scr[par, j] = s
                    m_run = jnp.maximum(m_run, s)
            if refill is not None:
                refill(js)
            return m_run, l_run, o_acc

        return lax.fori_loop(lo // unroll, hi // unroll, body, carry)

    def ahead(make, row_cur, row_next, j):
        jn = j + RD
        return make(jnp.where(jn < NC, row_cur, row_next), jnp.bitwise_and(jn, NC - 1))

    def run_unit(t, m_prev, kind):
        r_prev, r_cur, r_next = unit_row(t - 1), unit_row(t), unit_row(t + 1)
        carry = (jnp.full((8, CW), -jnp.inf, F32), jnp.zeros((8, CW), F32), jnp.zeros((8, PR), F32))
        do_qk = kind != 'last_pv'
        do_pv = kind != 'first'
        if kind == 'first':
            carry = chunk_loop(
                t, True, False, m_prev,
                lambda js: start_chunks(ahead(kch, r_cur, r_next, js[0]), vch(r_cur, js[0])), 1, 0, RD, carry)
            carry = chunk_loop(
                t, True, False, m_prev,
                lambda js: start_chunks(ahead(kch, r_cur, r_next, js[0]), ahead(kch, r_cur, r_next, js[1])),
                2, RD, NC, carry)
        elif kind == 'mid':
            carry = chunk_loop(
                t, True, True, m_prev,
                lambda js: start_chunks(ahead(vch, r_prev, r_cur, js[0]), ahead(kch, r_cur, r_next, js[0])),
                1, 0, NC, carry)
        elif kind == 'last_qk':
            carry = chunk_loop(
                t, True, True, m_prev,
                lambda js: start_chunks(kch(r_cur, js[0] + RD), vch(r_prev, js[0] + RD)), 1, 0, NC - RD, carry)
            carry = chunk_loop(
                t, True, True, m_prev,
                lambda js: start_chunks(vch(r_cur, js[0] + RD - NC), vch(r_cur, js[1] + RD - NC)),
                2, NC - RD, NC, carry)
        else:
            carry = chunk_loop(
                t, False, True, m_prev,
                lambda js: start_chunks(vch(r_prev, js[0] + RD), vch(r_prev, js[1] + RD)), 2, 0, NC - RD, carry)
            issue_ffn()
            carry = chunk_loop(t, False, True, m_prev, None, 2, NC - RD, NC, carry)
        m_run, l_run, o_acc = carry
        if do_pv:
            b = jnp.bitwise_and(t - 1, B - 1)
            g = lax.shift_right_logical(t - 1, 2)

            @pl.when(b == 0)
            def _():
                for p in range(NP):
                    wait(wo_piece(g, p))
            l = jnp.sum(l_run, axis=1, keepdims=True)
            o = jnp.where(bd_mask, o_acc / l, 0.0).astype(BF16)
            part = jnp.dot(o, wobuf[jnp.bitwise_and(g, 1)], preferred_element_type=F32)
            contrib = jnp.sum(part, axis=0, keepdims=True)
            rowa = lax.broadcasted_iota(jnp.int32, acc_scr.shape, 0)
            acc_scr[...] += jnp.where(rowa == b, jnp.broadcast_to(contrib, acc_scr.shape), 0.0)
        if do_qk:
            return jnp.broadcast_to(jnp.max(m_run, axis=1, keepdims=True), (8, CW))
        return m_prev

    def unit_head(t):
        g = lax.shift_right_logical(t, 2)

        @pl.when(jnp.bitwise_and(t, B - 1) == 0)
        def _():
            for p in range(NP):
                wait(wq_piece(g, p))
            q = jnp.dot(ln1_scr[...], wqbuf[jnp.bitwise_and(g, 1)], preferred_element_type=F32)
            q_scr[...] = q.astype(BF16).astype(F32)

    def unit_tail(t):
        g = lax.shift_right_logical(t, 2)
        b = jnp.bitwise_and(t, B - 1)
        g1 = lax.shift_right_logical(t + 1, 2)
        b1 = jnp.bitwise_and(t + 1, B - 1)

        @pl.when(g1 + 1 < NG)
        def _():
            start_pair(wq_piece(g1 + 1, b1), wo_piece(g + 1, b))

        @pl.when((b == B - 1) & (g1 + 1 < NG))
        def _():
            start_pair(wq_piece(g1 + 1, NP - 1), wo_piece(g + 1, NP - 1))

        @pl.when((b == B - 1) & (g1 + 1 == NG))
        def _():
            start_pair(wo_piece(g + 1, B - 1), wo_piece(g + 1, NP - 1))

    unit_head(0)
    m0 = run_unit(0, None, 'first')
    unit_tail(0)

    def outer(t, m_prev):
        unit_head(t)
        m = run_unit(t, m_prev, 'mid')
        unit_tail(t)
        return m

    m1 = lax.fori_loop(1, NU - 1, outer, m0)
    m2 = run_unit(NU - 1, m1, 'last_qk')
    run_unit(NU, m2, 'last_pv')

    cwr.wait()
    h = xbuf[...].astype(F32) + acc_scr[0:B, :]
    ln2 = _ln(h)
    ln2b = ln2.astype(BF16)
    r = jnp.sum(ln2b.astype(F32) * wrbuf[...].astype(F32)[None, :], axis=1, keepdims=True)
    pltpu.make_async_copy(wg_hbm, wgbuf, wsem.at[2]).wait()
    pltpu.make_async_copy(wu_hbm, wubuf, wsem.at[3]).wait()
    gt = jnp.dot(ln2b, wgbuf[...], preferred_element_type=F32)
    up = jnp.dot(ln2b, wubuf[...], preferred_element_type=F32)
    act = (gt * jax.nn.sigmoid(gt) * up).astype(BF16)
    y = jnp.zeros((B, D_MODEL), F32)
    for i in range(NWG):
        sl = pl.ds(i * PR, PR)
        pltpu.make_async_copy(wd_hbm.at[sl], wdbuf.at[sl], wdsem.at[i]).wait()
        y = y + jnp.dot(act[:, i * PR:(i + 1) * PR], wdbuf[sl, :], preferred_element_type=F32)
    out = h + (ln2 + y * jax.nn.sigmoid(r))
    out_ref[...] = out.astype(out_ref.dtype)


@jax.jit
def pallas_sequential_preLN__mha_block_cached__moe_arch_mod__decode_kernel(
    A_x, A_k_cache, A_v_cache, A_wq, A_wo, B_x, B_w_r, B_w_gate, B_w_up, B_w_down
):
    del B_x
    kt = jnp.swapaxes(A_k_cache, 2, 3).reshape(B * H * DH // 8, 8, SK)
    vt = jnp.swapaxes(A_v_cache, 2, 3).reshape(B * H * DH // 8, 8, SK)
    x2 = A_x.reshape(B, D_MODEL)
    anyspec = pl.BlockSpec(memory_space=pl.ANY)
    ring = pltpu.VMEM((RD, RT, 8, CW), BF16)
    out = pl.pallas_call(
        _kernel,
        in_specs=[anyspec] * 9,
        out_specs=pl.BlockSpec(memory_space=pltpu.VMEM),
        out_shape=jax.ShapeDtypeStruct((B, D_MODEL), BF16),
        scratch_shapes=[
            pltpu.VMEM((B, D_MODEL), BF16),
            pltpu.VMEM((D_MODEL,), BF16),
            pltpu.VMEM((B, D_MODEL), BF16),
            pltpu.VMEM((2, D_MODEL, PR), BF16),
            pltpu.VMEM((2, PR, D_MODEL), BF16),
            pltpu.VMEM((D_MODEL, FF), BF16),
            pltpu.VMEM((D_MODEL, FF), BF16),
            pltpu.VMEM((FF, D_MODEL), BF16),
            ring, ring,
            pltpu.VMEM((2, NC, 8, CW), F32),
            pltpu.VMEM((B, PR), F32),
            pltpu.VMEM((8, D_MODEL), F32),
            pltpu.SemaphoreType.DMA((RD,)),
            pltpu.SemaphoreType.DMA((RD,)),
            pltpu.SemaphoreType.DMA((4,)),
            pltpu.SemaphoreType.DMA((2,)),
            pltpu.SemaphoreType.DMA((2,)),
            pltpu.SemaphoreType.DMA((NWG,)),
        ],
        compiler_params=pltpu.CompilerParams(vmem_limit_bytes=64 * 1024 * 1024),
    )(x2, kt, vt, A_wq, A_wo, B_w_r, B_w_gate, B_w_up, B_w_down)
    return out.reshape(B, 1, D_MODEL)
```

```python
import jax
import jax.numpy as jnp
from jax import lax
from jax.experimental import pallas as pl
from jax.experimental.pallas import tpu as pltpu

B, D_MODEL, H, SK, DH, FF = 4, 640, 32, 8192, 192, 1536
CW = 128
NC = SK // CW
WP = 384
NP = D_MODEL // 128
NWG = FF // WP
HPU = 4
PR = HPU * DH
RT = PR // 8
NG = H // HPU
NU = B * NG
RD = 16
NS = 4
PPG = NP * (PR // WP)
PB = PPG // B
PX = PPG - B * PB
TA, TB = 0, 1
EPS = 1e-5
SCALE = DH ** -0.5
F32 = jnp.float32
BF16 = jnp.bfloat16


def _ln(x):
    m = jnp.mean(x, axis=-1, keepdims=True)
    xc = x - m
    v = jnp.mean(xc * xc, axis=-1, keepdims=True)
    return xc * lax.rsqrt(v + EPS)


def _kernel(x_hbm, k_hbm, v_hbm, wq_hbm, wo_hbm, wr_hbm, wg_hbm, wu_hbm, wd_hbm, out_ref,
            xbuf, wrbuf, ln1_scr, wqbuf, wobuf, wgbuf, wubuf, wdbuf, kbuf, vbuf, s_scr, q_scr, acc_scr,
            ksem, vsem, wsem, wqsem, wosem, wdsem):

    def unit_row(t):
        g = lax.shift_right_logical(t, 2)
        b = jnp.bitwise_and(t, B - 1)
        return b * (H * DH // 8) + g * RT

    def start_pair(a, b):
        for (src, dst, sem), prio in ((a, TA), (b, TB)):
            pltpu.make_async_copy(src, dst, sem).start(priority=prio)

    def start_chunks(a, b):
        rows = 8 // NS
        for i in range(NS):
            sl = (slice(None), pl.ds(i * rows, rows))
            start_pair((a[0].at[sl], a[1].at[sl], a[2]), (b[0].at[sl], b[1].at[sl], b[2]))

    def wait(d):
        pltpu.make_async_copy(*d).wait()

    def chunk(hbm, buf, sem, row, j):
        slot = jnp.bitwise_and(j, RD - 1)
        src = hbm.at[pl.ds(pl.multiple_of(row, RT), RT), :, pl.ds(pl.multiple_of(j * CW, CW), CW)]
        return src, buf.at[slot], sem.at[slot]

    def kch(row, j):
        return chunk(k_hbm, kbuf, ksem, row, j)

    def vch(row, j):
        return chunk(v_hbm, vbuf, vsem, row, j)

    def split(p):
        if isinstance(p, int):
            return p // NP, p % NP
        hi = lax.div(p, jnp.int32(NP))
        return hi, p - hi * NP

    def wq_piece(g, p):
        par = jnp.bitwise_and(g, 1)
        c, r = split(p)
        rows = pl.ds(pl.multiple_of(r * 128, 128), 128)
        return (wq_hbm.at[rows, pl.ds(pl.multiple_of(g * PR + c * WP, 128), WP)],
                wqbuf.at[par, rows, pl.ds(pl.multiple_of(c * WP, 128), WP)], wqsem.at[par])

    def wo_piece(g, p):
        par = jnp.bitwise_and(g, 1)
        r, c = split(p)
        cols = pl.ds(pl.multiple_of(c * 128, 128), 128)
        return (wo_hbm.at[pl.ds(pl.multiple_of(g * PR + r * WP, WP), WP), cols],
                wobuf.at[par, pl.ds(pl.multiple_of(r * WP, WP), WP), cols], wosem.at[par])

    def gu_piece(hbm, buf, sem, cg, p):
        sl = (pl.ds(pl.multiple_of(p * 128, 128), 128), pl.ds(pl.multiple_of(cg * WP, 128), WP))
        return hbm.at[sl], buf.at[sl], sem

    def wd_piece(rg, p):
        sl = (pl.ds(pl.multiple_of(rg * WP, WP), WP), pl.ds(pl.multiple_of(p * 128, 128), 128))
        return wd_hbm.at[sl], wdbuf.at[sl], wdsem.at[rg]

    cx = pltpu.make_async_copy(x_hbm, xbuf, wsem.at[0])
    cwr = pltpu.make_async_copy(wr_hbm, wrbuf, wsem.at[1])

    cx.start(priority=TB)

    def first_wq(p, c):
        start_pair(wq_piece(0, 2 * p), wq_piece(0, 2 * p + 1))
        return c
    lax.fori_loop(0, PPG // 2, first_wq, 0)

    row0 = unit_row(0)

    def fill(i, c):
        start_chunks(kch(row0, 2 * i), kch(row0, 2 * i + 1))
        return c
    lax.fori_loop(0, RD // 2, fill, 0)

    def first_wo(p, c):
        start_pair(wo_piece(0, 2 * p), wo_piece(0, 2 * p + 1))
        return c
    lax.fori_loop(0, PPG // 2, first_wo, 0)
    first_wq1 = list(range(PB)) + list(range(B * PB, PPG))
    for i in range(0, len(first_wq1), 2):
        start_pair(wq_piece(1, first_wq1[i]), wq_piece(1, first_wq1[i + 1]))
    cwr.start(priority=TA)

    cx.wait()
    ln1_scr[...] = _ln(xbuf[...].astype(F32)).astype(BF16)
    acc_scr[...] = jnp.zeros_like(acc_scr)

    row8 = lax.broadcasted_iota(jnp.int32, (8, PR), 0)
    lane8 = lax.broadcasted_iota(jnp.int32, (8, PR), 1)
    bd_mask = (lane8 >= row8 * DH) & (lane8 < (row8 + 1) * DH)

    def issue_ffn():
        def gate_up(cg, c):
            def piece(p, c2):
                start_pair(gu_piece(wg_hbm, wgbuf, wsem.at[2], cg, p), gu_piece(wu_hbm, wubuf, wsem.at[3], cg, p))
                return c2
            return lax.fori_loop(0, NP, piece, c)
        lax.fori_loop(0, FF // WP, gate_up, 0)

        def down(h2, c):
            def piece(p, c2):
                start_pair(wd_piece(2 * h2, p), wd_piece(2 * h2 + 1, p))
                return c2
            return lax.fori_loop(0, NP, piece, c)
        lax.fori_loop(0, NWG // 2, down, 0)

    def chunk_loop(t, do_qk, do_pv, m_prev, refill, unroll, lo, hi, carry):
        par = jnp.bitwise_and(t, 1)
        if do_qk:
            qrow = q_scr[pl.ds(jnp.bitwise_and(t, B - 1), 1), :]
            qbd = jnp.where(bd_mask, jnp.broadcast_to(qrow, (8, PR)), 0.0).astype(BF16)

        def body(jj, carry):
            m_run, l_run, o_acc = carry
            js = [jj * unroll + u for u in range(unroll)]
            slots = [jnp.bitwise_and(j, RD - 1) for j in js]
            for j in js:
                if do_qk:
                    wait(kch(0, j))
                if do_pv:
                    wait(vch(0, j))
            if do_pv:
                for j, slot in zip(js, slots):
                    p = jnp.exp((s_scr[1 - par, j] - m_prev) * SCALE)
                    l_run = l_run + p
                    o_acc = o_acc + lax.dot_general(
                        p.astype(BF16), vbuf[slot].reshape(PR, CW), (((1,), (1,)), ((), ())),
                        preferred_element_type=F32)
            if do_qk:
                for j, slot in zip(js, slots):
                    s = jnp.dot(qbd, kbuf[slot].reshape(PR, CW), preferred_element_type=F32)
                    s_scr[par, j] = s
                    m_run = jnp.maximum(m_run, s)
            if refill is not None:
                refill(js)
            return m_run, l_run, o_acc

        return lax.fori_loop(lo // unroll, hi // unroll, body, carry)

    def ahead(make, row_cur, row_next, j):
        jn = j + RD
        return make(jnp.where(jn < NC, row_cur, row_next), jnp.bitwise_and(jn, NC - 1))

    def run_unit(t, m_prev, kind):
        r_prev, r_cur, r_next = unit_row(t - 1), unit_row(t), unit_row(t + 1)
        carry = (jnp.full((8, CW), -jnp.inf, F32), jnp.zeros((8, CW), F32), jnp.zeros((8, PR), F32))
        do_qk = kind != 'last_pv'
        do_pv = kind != 'first'
        if kind == 'first':
            carry = chunk_loop(
                t, True, False, m_prev,
                lambda js: start_chunks(ahead(kch, r_cur, r_next, js[0]), vch(r_cur, js[0])), 1, 0, RD, carry)
            carry = chunk_loop(
                t, True, False, m_prev,
                lambda js: start_chunks(ahead(kch, r_cur, r_next, js[0]), ahead(kch, r_cur, r_next, js[1])),
                2, RD, NC, carry)
        elif kind == 'mid':
            carry = chunk_loop(
                t, True, True, m_prev,
                lambda js: start_chunks(ahead(kch, r_cur, r_next, js[0]), ahead(vch, r_prev, r_cur, js[0])),
                1, 0, NC, carry)
        elif kind == 'last_qk':
            carry = chunk_loop(
                t, True, True, m_prev,
                lambda js: start_chunks(kch(r_cur, js[0] + RD), vch(r_prev, js[0] + RD)), 1, 0, NC - RD, carry)
            carry = chunk_loop(
                t, True, True, m_prev,
                lambda js: start_chunks(vch(r_cur, js[0] + RD - NC), vch(r_cur, js[1] + RD - NC)),
                2, NC - RD, NC, carry)
        else:
            carry = chunk_loop(
                t, False, True, m_prev,
                lambda js: start_chunks(vch(r_prev, js[0] + RD), vch(r_prev, js[1] + RD)), 2, 0, NC - RD, carry)
            issue_ffn()
            carry = chunk_loop(t, False, True, m_prev, None, 2, NC - RD, NC, carry)
        m_run, l_run, o_acc = carry
        if do_pv:
            b = jnp.bitwise_and(t - 1, B - 1)
            g = lax.shift_right_logical(t - 1, 2)

            @pl.when(b == 0)
            def _():
                for p in range(PPG):
                    wait(wo_piece(g, p))
            l = jnp.sum(l_run, axis=1, keepdims=True)
            o = jnp.where(bd_mask, o_acc / l, 0.0).astype(BF16)
            part = jnp.dot(o, wobuf[jnp.bitwise_and(g, 1)], preferred_element_type=F32)
            contrib = jnp.sum(part, axis=0, keepdims=True)
            rowa = lax.broadcasted_iota(jnp.int32, acc_scr.shape, 0)
            acc_scr[...] += jnp.where(rowa == b, jnp.broadcast_to(contrib, acc_scr.shape), 0.0)
        if do_qk:
            return jnp.broadcast_to(jnp.max(m_run, axis=1, keepdims=True), (8, CW))
        return m_prev

    def unit_head(t):
        g = lax.shift_right_logical(t, 2)

        @pl.when(jnp.bitwise_and(t, B - 1) == 0)
        def _():
            for p in range(PPG):
                wait(wq_piece(g, p))
            q = jnp.dot(ln1_scr[...], wqbuf[jnp.bitwise_and(g, 1)], preferred_element_type=F32)
            q_scr[...] = q.astype(BF16).astype(F32)

    def unit_tail(t):
        g = lax.shift_right_logical(t, 2)
        b = jnp.bitwise_and(t, B - 1)
        g1 = lax.shift_right_logical(t + 1, 2)
        b1 = jnp.bitwise_and(t + 1, B - 1)

        @pl.when(g1 + 1 < NG)
        def _():
            for i in range(PB):
                start_pair(wq_piece(g1 + 1, PB * b1 + i), wo_piece(g + 1, PB * b + i))

        @pl.when((b == B - 1) & (g1 + 1 < NG))
        def _():
            for i in range(PX):
                start_pair(wq_piece(g1 + 1, B * PB + i), wo_piece(g + 1, B * PB + i))

        @pl.when((b == B - 1) & (g1 + 1 == NG))
        def _():
            rest = list(range((B - 1) * PB, PPG))
            for i in range(0, len(rest), 2):
                start_pair(wo_piece(g + 1, rest[i]), wo_piece(g + 1, rest[i + 1]))

    unit_head(0)
    m0 = run_unit(0, None, 'first')
    unit_tail(0)

    def outer(t, m_prev):
        unit_head(t)
        m = run_unit(t, m_prev, 'mid')
        unit_tail(t)
        return m

    m1 = lax.fori_loop(1, NU - 1, outer, m0)
    m2 = run_unit(NU - 1, m1, 'last_qk')
    run_unit(NU, m2, 'last_pv')

    cwr.wait()
    h = xbuf[...].astype(F32) + acc_scr[0:B, :]
    ln2 = _ln(h)
    ln2b = ln2.astype(BF16)
    r = jnp.sum(ln2b.astype(F32) * wrbuf[...].astype(F32)[None, :], axis=1, keepdims=True)
    pltpu.make_async_copy(wg_hbm, wgbuf, wsem.at[2]).wait()
    pltpu.make_async_copy(wu_hbm, wubuf, wsem.at[3]).wait()
    gt = jnp.dot(ln2b, wgbuf[...], preferred_element_type=F32)
    up = jnp.dot(ln2b, wubuf[...], preferred_element_type=F32)
    act = (gt * jax.nn.sigmoid(gt) * up).astype(BF16)
    y = jnp.zeros((B, D_MODEL), F32)
    for i in range(NWG):
        sl = pl.ds(i * WP, WP)
        pltpu.make_async_copy(wd_hbm.at[sl], wdbuf.at[sl], wdsem.at[i]).wait()
        y = y + jnp.dot(act[:, i * WP:(i + 1) * WP], wdbuf[sl, :], preferred_element_type=F32)
    out = h + (ln2 + y * jax.nn.sigmoid(r))
    out_ref[...] = out.astype(out_ref.dtype)


@jax.jit
def pallas_sequential_preLN__mha_block_cached__moe_arch_mod__decode_kernel(
    A_x, A_k_cache, A_v_cache, A_wq, A_wo, B_x, B_w_r, B_w_gate, B_w_up, B_w_down
):
    del B_x
    kt = jnp.swapaxes(A_k_cache, 2, 3).reshape(B * H * DH // 8, 8, SK)
    vt = jnp.swapaxes(A_v_cache, 2, 3).reshape(B * H * DH // 8, 8, SK)
    x2 = A_x.reshape(B, D_MODEL)
    anyspec = pl.BlockSpec(memory_space=pl.ANY)
    ring = pltpu.VMEM((RD, RT, 8, CW), BF16)
    out = pl.pallas_call(
        _kernel,
        in_specs=[anyspec] * 9,
        out_specs=pl.BlockSpec(memory_space=pltpu.VMEM),
        out_shape=jax.ShapeDtypeStruct((B, D_MODEL), BF16),
        scratch_shapes=[
            pltpu.VMEM((B, D_MODEL), BF16),
            pltpu.VMEM((D_MODEL,), BF16),
            pltpu.VMEM((B, D_MODEL), BF16),
            pltpu.VMEM((2, D_MODEL, PR), BF16),
            pltpu.VMEM((2, PR, D_MODEL), BF16),
            pltpu.VMEM((D_MODEL, FF), BF16),
            pltpu.VMEM((D_MODEL, FF), BF16),
            pltpu.VMEM((FF, D_MODEL), BF16),
            ring, ring,
            pltpu.VMEM((2, NC, 8, CW), F32),
            pltpu.VMEM((B, PR), F32),
            pltpu.VMEM((8, D_MODEL), F32),
            pltpu.SemaphoreType.DMA((RD,)),
            pltpu.SemaphoreType.DMA((RD,)),
            pltpu.SemaphoreType.DMA((4,)),
            pltpu.SemaphoreType.DMA((2,)),
            pltpu.SemaphoreType.DMA((2,)),
            pltpu.SemaphoreType.DMA((NWG,)),
        ],
        compiler_params=pltpu.CompilerParams(vmem_limit_bytes=64 * 1024 * 1024),
    )(x2, kt, vt, A_wq, A_wo, B_w_r, B_w_gate, B_w_up, B_w_down)
    return out.reshape(B, 1, D_MODEL)
```

```python
import jax
import jax.numpy as jnp
from jax import lax
from jax.experimental import pallas as pl
from jax.experimental.pallas import tpu as pltpu

B, D_MODEL, H, SK, DH, FF = 4, 640, 32, 8192, 192, 1536
CW = 128
NC = SK // CW
NT = B * H * DH // 8
HG = 8
GR = HG * DH
GT = GR // 8
NG = NT // GT
GPB = H // HG
RT = 64
DPG = GT // RT
NS = 4
SPP = NG // NS
PPS = (NT // RT) // SPP
WP = 384
NP = D_MODEL // 128
NWG = FF // WP
PPG = NP * (GR // WP)
TAIL_PER_STEP = 4
TA, TB = 0, 1
EPS = 1e-5
SCALE = DH ** -0.5
F32 = jnp.float32
BF16 = jnp.bfloat16


def _ln(x):
    m = jnp.mean(x, axis=-1, keepdims=True)
    xc = x - m
    v = jnp.mean(xc * xc, axis=-1, keepdims=True)
    return xc * lax.rsqrt(v + EPS)


def _kernel(x_hbm, k_hbm, v_hbm, wq_hbm, wo_hbm, wr_hbm, wg_hbm, wu_hbm, wd_hbm, out_ref,
            xbuf, wrbuf, wqbuf, wobuf, wgbuf, wubuf, wdbuf, kbuf, vbuf, qbd_scr, m_scr, l_scr, o_scr,
            ksem, vsem, wsem, wqsem, wosem, wdsem):

    def start_pair(a, b):
        for (src, dst, sem), prio in ((a, TA), (b, TB)):
            pltpu.make_async_copy(src, dst, sem).start(priority=prio)

    def wait(d):
        pltpu.make_async_copy(*d).wait()

    def col_slice(c):
        return pl.ds(pl.multiple_of(c * CW, CW), CW)

    def issue_kv(c, s, i):
        slot = jnp.bitwise_and(c, 1)
        col = col_slice(c)
        sub = pl.ds(s * 2, 2)
        for q in range(PPS):
            rows = pl.ds((i * PPS + q) * RT, RT)
            g = i * (PPS // DPG) + q // DPG
            start_pair((k_hbm.at[rows, sub, col], kbuf.at[slot, rows, sub], ksem.at[slot, g]),
                       (v_hbm.at[rows, sub, col], vbuf.at[slot, rows, sub], vsem.at[slot, g]))

    def group(hbm, buf, sem, c, g):
        slot = jnp.bitwise_and(c, 1)
        rows = pl.ds(g * GT, GT)
        return hbm.at[rows, :, col_slice(c)], buf.at[slot, rows], sem.at[slot, g]

    def wq_piece(gg, p):
        c, r = p // NP, p % NP
        sl = (pl.ds(r * 128, 128), pl.ds(gg * GR + c * WP, WP))
        return wq_hbm.at[sl], wqbuf.at[sl], wqsem.at[gg]

    def wo_piece(gg, p):
        r, c = p // NP, p % NP
        sl = (pl.ds(gg * GR + r * WP, WP), pl.ds(c * 128, 128))
        return wo_hbm.at[sl], wobuf.at[sl], wosem.at[gg]

    def gu_piece(hbm, buf, sem, cg, p):
        sl = (pl.ds(p * 128, 128), pl.ds(cg * WP, WP))
        return hbm.at[sl], buf.at[sl], sem

    def wd_piece(rg, p):
        sl = (pl.ds(rg * WP, WP), pl.ds(p * 128, 128))
        return wd_hbm.at[sl], wdbuf.at[sl], wdsem.at[rg]

    tail = []
    for gg in range(GPB):
        for p in range(0, PPG, 2):
            tail.append((wo_piece, (gg, p), wo_piece, (gg, p + 1)))
    for cg in range(FF // WP):
        for p in range(NP):
            tail.append((gu_piece, (wg_hbm, wgbuf, wsem.at[2], cg, p), gu_piece, (wu_hbm, wubuf, wsem.at[3], cg, p)))
    for h2 in range(NWG // 2):
        for p in range(NP):
            tail.append((wd_piece, (2 * h2, p), wd_piece, (2 * h2 + 1, p)))

    def issue_tail(lo, hi):
        for fa, aa, fb, ab in tail[lo:hi]:
            start_pair(fa(*aa), fb(*ab))

    cx = pltpu.make_async_copy(x_hbm, xbuf, wsem.at[0])
    cwr = pltpu.make_async_copy(wr_hbm, wrbuf, wsem.at[1])

    row8 = lax.broadcasted_iota(jnp.int32, (8, GR), 0)
    lane8 = lax.broadcasted_iota(jnp.int32, (8, GR), 1)
    bd_mask = (lane8 >= row8 * DH) & (lane8 < (row8 + 1) * DH)

    cx.start(priority=TB)
    cwr.start(priority=TA)
    for gg in range(GPB):
        for p in range(0, PPG, 2):
            start_pair(wq_piece(gg, p), wq_piece(gg, p + 1))

    def pass_loop(c, s, lo, hi):
        def f(i, carry):
            issue_kv(c, s, i)
            return carry
        lax.fori_loop(lo, hi, f, 0)

    pass_loop(0, 0, 0, SPP)
    cx.wait()
    ln1 = _ln(xbuf[...].astype(F32)).astype(BF16)
    m_scr[...] = jnp.full(m_scr.shape, -jnp.inf, F32)
    l_scr[...] = jnp.zeros(l_scr.shape, F32)
    o_scr[...] = jnp.zeros(o_scr.shape, F32)
    for gg in range(GPB):
        wait((wq_hbm.at[:, pl.ds(gg * GR, GR)], wqbuf.at[:, pl.ds(gg * GR, GR)], wqsem.at[gg]))
        q = jnp.dot(ln1, wqbuf[:, gg * GR:(gg + 1) * GR], preferred_element_type=F32)
        for b in range(B):
            qb = jnp.broadcast_to(q[b:b + 1, :], (8, GR))
            qbd_scr[b * GPB + gg] = jnp.where(bd_mask, qb, 0.0).astype(BF16)
        issue_kv(0, 1, gg)
    pass_loop(0, 2, 0, SPP)
    pass_loop(0, 3, 0, SPP)

    def step(c, g):
        slot = jnp.bitwise_and(c, 1)
        rows = pl.ds(g * GT, GT)
        wait(group(k_hbm, kbuf, ksem, c, g))
        s = jnp.dot(qbd_scr[g], kbuf[slot, rows].reshape(GR, CW), preferred_element_type=F32)
        m_old = m_scr[g]
        m_new = jnp.maximum(m_old, jnp.broadcast_to(jnp.max(s, axis=1, keepdims=True), (8, CW)))
        alpha = jnp.exp((m_old - m_new) * SCALE)
        p = jnp.exp((s - m_new) * SCALE)
        m_scr[g] = m_new
        l_scr[g] = l_scr[g] * alpha + p
        wait(group(v_hbm, vbuf, vsem, c, g))
        pv = lax.dot_general(p.astype(BF16), vbuf[slot, rows].reshape(GR, CW), (((1,), (1,)), ((), ())),
                             preferred_element_type=F32)
        o_scr[g] = o_scr[g] * alpha[:, 0:1] + pv

    def column(c, carry):
        for s in range(NS):
            def st(i, c2, s=s):
                step(c, s * SPP + i)
                issue_kv(c + 1, s, i)
                return c2
            lax.fori_loop(0, SPP, st, 0, unroll=2)
        return carry

    lax.fori_loop(0, NC - 1, column, 0)

    ntail = len(tail)
    per = TAIL_PER_STEP
    for g in range(NG):
        issue_tail(min(g * per, ntail), min((g + 1) * per, ntail))
        step(NC - 1, g)
    issue_tail(min(NG * per, ntail), ntail)

    rowa = lax.broadcasted_iota(jnp.int32, (8, GR), 0)
    attn = jnp.zeros((8, D_MODEL), F32)
    for gg in range(GPB):
        oin = jnp.zeros((8, GR), F32)
        for b in range(B):
            g = b * GPB + gg
            l = jnp.sum(l_scr[g], axis=1, keepdims=True)
            o = jnp.where(bd_mask, o_scr[g] / l, 0.0)
            orow = jnp.sum(o, axis=0, keepdims=True)
            oin = jnp.where(rowa == b, jnp.broadcast_to(orow, (8, GR)), oin)
        sl = pl.ds(gg * GR, GR)
        wait((wo_hbm.at[sl], wobuf.at[sl], wosem.at[gg]))
        attn = attn + jnp.dot(oin.astype(BF16), wobuf[sl, :], preferred_element_type=F32)

    cwr.wait()
    h = xbuf[...].astype(F32) + attn[0:B, :]
    ln2 = _ln(h)
    ln2b = ln2.astype(BF16)
    r = jnp.sum(ln2b.astype(F32) * wrbuf[...].astype(F32)[None, :], axis=1, keepdims=True)
    pltpu.make_async_copy(wg_hbm, wgbuf, wsem.at[2]).wait()
    pltpu.make_async_copy(wu_hbm, wubuf, wsem.at[3]).wait()
    gt = jnp.dot(ln2b, wgbuf[...], preferred_element_type=F32)
    up = jnp.dot(ln2b, wubuf[...], preferred_element_type=F32)
    act = (gt * jax.nn.sigmoid(gt) * up).astype(BF16)
    y = jnp.zeros((B, D_MODEL), F32)
    for i in range(NWG):
        sl = pl.ds(i * WP, WP)
        pltpu.make_async_copy(wd_hbm.at[sl], wdbuf.at[sl], wdsem.at[i]).wait()
        y = y + jnp.dot(act[:, i * WP:(i + 1) * WP], wdbuf[sl, :], preferred_element_type=F32)
    out = h + (ln2 + y * jax.nn.sigmoid(r))
    out_ref[...] = out.astype(out_ref.dtype)


@jax.jit
def pallas_sequential_preLN__mha_block_cached__moe_arch_mod__decode_kernel(
    A_x, A_k_cache, A_v_cache, A_wq, A_wo, B_x, B_w_r, B_w_gate, B_w_up, B_w_down
):
    del B_x
    kt = jnp.swapaxes(A_k_cache, 2, 3).reshape(NT, 8, SK)
    vt = jnp.swapaxes(A_v_cache, 2, 3).reshape(NT, 8, SK)
    x2 = A_x.reshape(B, D_MODEL)
    anyspec = pl.BlockSpec(memory_space=pl.ANY)
    ring = pltpu.VMEM((2, NT, 8, CW), BF16)
    out = pl.pallas_call(
        _kernel,
        in_specs=[anyspec] * 9,
        out_specs=pl.BlockSpec(memory_space=pltpu.VMEM),
        out_shape=jax.ShapeDtypeStruct((B, D_MODEL), BF16),
        scratch_shapes=[
            pltpu.VMEM((B, D_MODEL), BF16),
            pltpu.VMEM((D_MODEL,), BF16),
            pltpu.VMEM((D_MODEL, H * DH), BF16),
            pltpu.VMEM((H * DH, D_MODEL), BF16),
            pltpu.VMEM((D_MODEL, FF), BF16),
            pltpu.VMEM((D_MODEL, FF), BF16),
            pltpu.VMEM((FF, D_MODEL), BF16),
            ring, ring,
            pltpu.VMEM((NG, 8, GR), BF16),
            pltpu.VMEM((NG, 8, CW), F32),
            pltpu.VMEM((NG, 8, CW), F32),
            pltpu.VMEM((NG, 8, GR), F32),
            pltpu.SemaphoreType.DMA((2, NG)),
            pltpu.SemaphoreType.DMA((2, NG)),
            pltpu.SemaphoreType.DMA((4,)),
            pltpu.SemaphoreType.DMA((GPB,)),
            pltpu.SemaphoreType.DMA((GPB,)),
            pltpu.SemaphoreType.DMA((NWG,)),
        ],
        compiler_params=pltpu.CompilerParams(vmem_limit_bytes=100 * 1024 * 1024),
    )(x2, kt, vt, A_wq, A_wo, B_w_r, B_w_gate, B_w_up, B_w_down)
    return out.reshape(B, 1, D_MODEL)
```

```python
import jax
import jax.numpy as jnp
from jax import lax
from jax.experimental import pallas as pl
from jax.experimental.pallas import tpu as pltpu

B, D_MODEL, H, SK, DH, FF = 4, 640, 32, 8192, 192, 1536
CW = 128
NC = SK // CW
NA = B * H * DH // 16
HG = 8
GR = HG * DH
GA = GR // 16
NG = NA // GA
GPB = H // HG
RT = 64
NS = 4
NAB = NA // RT
SGA = 2 * GA
NSG = NA // SGA
ABS = SGA // RT
NR = 3
WQ_R, WQ_C = 8, 2048
WO_R = 32
GU_R = 16
NGU = 5
NWD = 4
TAIL_PER_STEP = 14
TAIL_PER_SLICE = (0, 10, 20, 20)
TA, TB = 0, 1
EPS = 1e-5
SCALE = DH ** -0.5
F32 = jnp.float32
BF16 = jnp.bfloat16


def _ln(x):
    m = jnp.mean(x, axis=-1, keepdims=True)
    xc = x - m
    v = jnp.mean(xc * xc, axis=-1, keepdims=True)
    return xc * lax.rsqrt(v + EPS)


def _scattered(n, m):
    return [(k * m) % n for k in range(n)]


def _kernel(x_hbm, k_hbm, v_hbm, wq_hbm, wo_hbm, wr_hbm, wg_hbm, wu_hbm, wd_hbm, out_ref,
            xbuf, wrbuf, wqbuf, wobuf, wgbuf, wubuf, wdbuf, kbuf, vbuf, qbd_scr, m_scr, l_scr, o_scr,
            ksem, vsem, wsem, wosem, gusem, wdsem):

    def start_pair(a, b):
        for (src, dst, sem), prio in ((a, TA), (b, TB)):
            pltpu.make_async_copy(src, dst, sem).start(priority=prio)

    def wait(d):
        pltpu.make_async_copy(*d).wait()

    def col_slice(c):
        return pl.ds(pl.multiple_of(c * CW, CW), CW)

    def issue_kv(c, s, par):
        slot = lax.rem(c, jnp.int32(NR))
        col = col_slice(c)
        sub = pl.ds(s * 2, 2)
        for ab in range(NAB):
            rows = pl.ds(ab * RT, RT)
            start_pair((k_hbm.at[rows, par, sub, col], kbuf.at[slot, rows, par, sub], ksem.at[slot, ab // ABS]),
                       (v_hbm.at[rows, par, sub, col], vbuf.at[slot, rows, par, sub], vsem.at[slot, ab // ABS]))

    def issue_pass(c, s):
        def f(par, carry):
            issue_kv(c, s, par)
            return carry
        lax.fori_loop(0, 2, f, 0)

    def sgroup(hbm, buf, sem, c, sg):
        slot = lax.rem(c, jnp.int32(NR))
        rows = pl.ds(sg * SGA, SGA)
        return hbm.at[rows, :, :, col_slice(c)], buf.at[slot, rows], sem.at[slot, sg]

    def piece(hbm, buf, sem, r0, rn, c0, cn):
        sl = (pl.ds(r0, rn), pl.ds(c0, cn))
        return hbm.at[sl], buf.at[sl], sem

    wq_pos = [(r, c) for r in range(0, D_MODEL, WQ_R) for c in range(0, H * DH, WQ_C)]
    wq_list = [piece(wq_hbm, wqbuf, wsem.at[2], wq_pos[k][0], WQ_R, wq_pos[k][1], WQ_C)
               for k in _scattered(len(wq_pos), 11)]

    gur = D_MODEL // NGU
    wdr = FF // NWD
    tail = []
    for gg in range(GPB):
        for k in _scattered(GR // WO_R, 7):
            tail.append(piece(wo_hbm, wobuf, wosem.at[gg], gg * GR + k * WO_R, WO_R, 0, D_MODEL))
    for i in range(NGU):
        for k in range(gur // GU_R):
            tail.append(piece(wg_hbm, wgbuf, gusem.at[i], i * gur + k * GU_R, GU_R, 0, FF))
            tail.append(piece(wu_hbm, wubuf, gusem.at[i], i * gur + k * GU_R, GU_R, 0, FF))
    for i in range(NWD):
        for k in _scattered(wdr // WO_R, 5):
            tail.append(piece(wd_hbm, wdbuf, wdsem.at[i], i * wdr + k * WO_R, WO_R, 0, D_MODEL))
    tail_pos = [0]

    def issue_tail(n):
        lo = tail_pos[0]
        hi = min(lo + 2 * n, len(tail))
        for k in range(lo, hi, 2):
            start_pair(tail[k], tail[k + 1])
        tail_pos[0] = hi

    cx = pltpu.make_async_copy(x_hbm, xbuf, wsem.at[0])
    cwr = pltpu.make_async_copy(wr_hbm, wrbuf, wsem.at[1])

    row8 = lax.broadcasted_iota(jnp.int32, (8, GR), 0)
    lane8 = lax.broadcasted_iota(jnp.int32, (8, GR), 1)
    bd_mask = (lane8 >= row8 * DH) & (lane8 < (row8 + 1) * DH)

    cx.start(priority=TB)
    cwr.start(priority=TA)
    for k in range(0, len(wq_list), 2):
        start_pair(wq_list[k], wq_list[k + 1])
    issue_pass(0, 0)
    cx.wait()
    ln1 = _ln(xbuf[...].astype(F32)).astype(BF16)
    m_scr[...] = jnp.full(m_scr.shape, -jnp.inf, F32)
    l_scr[...] = jnp.zeros(l_scr.shape, F32)
    o_scr[...] = jnp.zeros(o_scr.shape, F32)
    wait((wq_hbm, wqbuf, wsem.at[2]))
    for gg in range(GPB):
        q = jnp.dot(ln1, wqbuf[:, gg * GR:(gg + 1) * GR], preferred_element_type=F32)
        for b in range(B):
            qb = jnp.broadcast_to(q[b:b + 1, :], (8, GR))
            qbd_scr[b * GPB + gg] = jnp.where(bd_mask, qb, 0.0).astype(BF16)
        if gg % 2 == 1:
            issue_kv(0, 1, gg // 2)
    issue_pass(0, 2)
    issue_pass(0, 3)
    issue_pass(1, 0)

    def step(c, g):
        slot = lax.rem(c, jnp.int32(NR))
        rows = pl.ds(g * GA, GA)
        s = jnp.dot(qbd_scr[g], kbuf[slot, rows].reshape(GR, CW), preferred_element_type=F32)
        m_old = m_scr[g]
        m_new = jnp.maximum(m_old, jnp.broadcast_to(jnp.max(s, axis=1, keepdims=True), (8, CW)))
        alpha = jnp.exp((m_old - m_new) * SCALE)
        p = jnp.exp((s - m_new) * SCALE)
        m_scr[g] = m_new
        l_scr[g] = l_scr[g] * alpha + p
        pv = lax.dot_general(p.astype(BF16), vbuf[slot, rows].reshape(GR, CW), (((1,), (1,)), ((), ())),
                             preferred_element_type=F32)
        o_scr[g] = o_scr[g] * alpha[:, 0:1] + pv

    def super_step(c, sg):
        wait(sgroup(k_hbm, kbuf, ksem, c, sg))
        wait(sgroup(v_hbm, vbuf, vsem, c, sg))
        step(c, 2 * sg)
        step(c, 2 * sg + 1)

    def quarter(c, s):
        def body(i, carry):
            super_step(c, 2 * s + i)
            issue_kv(c + 1 + (s + 1) // NS, (s + 1) % NS, i)
            return carry
        lax.fori_loop(0, 2, body, 0)

    def column(c, carry):
        for s in range(NS):
            quarter(c, s)
        return carry

    lax.fori_loop(0, NC - 2, column, 0)
    for s in range(NS - 1):
        quarter(NC - 2, s)
    for c, sg in [(NC - 2, NSG - 2), (NC - 2, NSG - 1)] + [(NC - 1, k) for k in range(NSG)]:
        super_step(c, sg)
        issue_tail(TAIL_PER_STEP)

    attn = jnp.zeros((8, D_MODEL), F32)
    for gg in range(GPB):
        issue_tail(TAIL_PER_SLICE[gg])
        oin = jnp.zeros((8, GR), F32)
        for b in range(B):
            g = b * GPB + gg
            l = jnp.sum(l_scr[g], axis=1, keepdims=True)
            o = jnp.where(bd_mask, o_scr[g] / l, 0.0)
            orow = jnp.sum(o, axis=0, keepdims=True)
            oin = jnp.where(row8 == b, jnp.broadcast_to(orow, (8, GR)), oin)
        sl = pl.ds(gg * GR, GR)
        wait((wo_hbm.at[sl], wobuf.at[sl], wosem.at[gg]))
        attn = attn + jnp.dot(oin.astype(BF16), wobuf[sl, :], preferred_element_type=F32)

    cwr.wait()
    h = xbuf[...].astype(F32) + attn[0:B, :]
    ln2 = _ln(h)
    ln2b = ln2.astype(BF16)
    r = jnp.sum(ln2b.astype(F32) * wrbuf[...].astype(F32)[None, :], axis=1, keepdims=True)
    issue_tail(len(tail))
    gt = jnp.zeros((B, FF), F32)
    up = jnp.zeros((B, FF), F32)
    for i in range(NGU):
        sl = pl.ds(i * gur, gur)
        wait((wg_hbm.at[sl], wgbuf.at[sl], gusem.at[i]))
        wait((wu_hbm.at[sl], wubuf.at[sl], gusem.at[i]))
        lhs = ln2b[:, i * gur:(i + 1) * gur]
        gt = gt + jnp.dot(lhs, wgbuf[sl, :], preferred_element_type=F32)
        up = up + jnp.dot(lhs, wubuf[sl, :], preferred_element_type=F32)
    act = (gt * jax.nn.sigmoid(gt) * up).astype(BF16)
    y = jnp.zeros((B, D_MODEL), F32)
    for i in range(NWD):
        sl = pl.ds(i * wdr, wdr)
        wait((wd_hbm.at[sl], wdbuf.at[sl], wdsem.at[i]))
        y = y + jnp.dot(act[:, i * wdr:(i + 1) * wdr], wdbuf[sl, :], preferred_element_type=F32)
    out = h + (ln2 + y * jax.nn.sigmoid(r))
    out_ref[...] = out.astype(out_ref.dtype)


@jax.jit
def pallas_sequential_preLN__mha_block_cached__moe_arch_mod__decode_kernel(
    A_x, A_k_cache, A_v_cache, A_wq, A_wo, B_x, B_w_r, B_w_gate, B_w_up, B_w_down
):
    del B_x
    kt = jnp.swapaxes(A_k_cache, 2, 3).reshape(NA, 2, 8, SK)
    vt = jnp.swapaxes(A_v_cache, 2, 3).reshape(NA, 2, 8, SK)
    x2 = A_x.reshape(B, D_MODEL)
    anyspec = pl.BlockSpec(memory_space=pl.ANY)
    ring = pltpu.VMEM((NR, NA, 2, 8, CW), BF16)
    out = pl.pallas_call(
        _kernel,
        in_specs=[anyspec] * 9,
        out_specs=pl.BlockSpec(memory_space=pltpu.VMEM),
        out_shape=jax.ShapeDtypeStruct((B, D_MODEL), BF16),
        scratch_shapes=[
            pltpu.VMEM((B, D_MODEL), BF16),
            pltpu.VMEM((D_MODEL,), BF16),
            pltpu.VMEM((D_MODEL, H * DH), BF16),
            pltpu.VMEM((H * DH, D_MODEL), BF16),
            pltpu.VMEM((D_MODEL, FF), BF16),
            pltpu.VMEM((D_MODEL, FF), BF16),
            pltpu.VMEM((FF, D_MODEL), BF16),
            ring, ring,
            pltpu.VMEM((NG, 8, GR), BF16),
            pltpu.VMEM((NG, 8, CW), F32),
            pltpu.VMEM((NG, 8, CW), F32),
            pltpu.VMEM((NG, 8, GR), F32),
            pltpu.SemaphoreType.DMA((NR, NSG)),
            pltpu.SemaphoreType.DMA((NR, NSG)),
            pltpu.SemaphoreType.DMA((3,)),
            pltpu.SemaphoreType.DMA((GPB,)),
            pltpu.SemaphoreType.DMA((NGU,)),
            pltpu.SemaphoreType.DMA((NWD,)),
        ],
        compiler_params=pltpu.CompilerParams(vmem_limit_bytes=100 * 1024 * 1024),
    )(x2, kt, vt, A_wq, A_wo, B_w_r, B_w_gate, B_w_up, B_w_down)
    return out.reshape(B, 1, D_MODEL)
```

```python
import jax
import jax.numpy as jnp
from jax import lax
from jax.experimental import pallas as pl
from jax.experimental.pallas import tpu as pltpu

B, D_MODEL, H, SK, DH, FF = 4, 640, 32, 8192, 192, 1536
CW = 128
NC = SK // CW
NA = B * H * DH // 16
HG = 8
GR = HG * DH
GA = GR // 16
NG = NA // GA
GPB = H // HG
RT = 64
NS = 4
NAB = NA // RT
NR = 3
NQ = 2
NSS = NG // 2
AHEAD = NSS + 2
WQ_R, WQ_C = 8, 2048
WO_R = 32
GU_R = 16
WO_PER_STEP = 16
GU_GROUPS = (256, 256, 128)
WD_GROUPS = (512, 512, 512)
TAIL_PER_SLICE = (24, 12, 12, 12)
TA, TB = 0, 1
EPS = 1e-5
SCALE = DH ** -0.5
F32 = jnp.float32
BF16 = jnp.bfloat16


def _ln(x):
    m = jnp.mean(x, axis=-1, keepdims=True)
    xc = x - m
    v = jnp.mean(xc * xc, axis=-1, keepdims=True)
    return xc * lax.rsqrt(v + EPS)


def _scattered(n, m):
    return [(k * m) % n for k in range(n)]


def _kernel(x_hbm, k_hbm, v_hbm, wq_hbm, wo_hbm, wr_hbm, wg_hbm, wu_hbm, wd_hbm, out_ref,
            xbuf, wrbuf, wqbuf, wobuf, wgbuf, wubuf, wdbuf, kbuf, vbuf, qbd_scr, m_scr, l_scr, o_scr,
            kvsem, wsem):

    def start_pair(a, b):
        for (src, dst, sem), prio in ((a, TA), (b, TB)):
            pltpu.make_async_copy(src, dst, sem).start(priority=prio)

    def wait(d):
        pltpu.make_async_copy(*d).wait()

    def col_slice(c):
        return pl.ds(pl.multiple_of(c * CW, CW), CW)

    def issue_kv(c, s, par):
        slot = lax.rem(c, jnp.int32(NR))
        col = col_slice(c)
        sub = pl.ds(s * 2, 2)
        for ab in range(NAB):
            rows = pl.ds(ab * RT, RT)
            sem = kvsem.at[slot, ab // (NAB // NQ)]
            start_pair((k_hbm.at[rows, par, sub, col], kbuf.at[slot, rows, par, sub], sem),
                       (v_hbm.at[rows, par, sub, col], vbuf.at[slot, rows, par, sub], sem))

    def issue_pass(c, s):
        def f(par, carry):
            issue_kv(c, s, par)
            return carry
        lax.fori_loop(0, 2, f, 0)

    def kv_part(hbm, buf, c, q):
        slot = lax.rem(c, jnp.int32(NR))
        rows = pl.ds(q * (NA // NQ), NA // NQ)
        return hbm.at[rows, :, :, col_slice(c)], buf.at[slot, rows], kvsem.at[slot, q]

    def piece(hbm, buf, sem, r0, rn, c0, cn):
        sl = (pl.ds(r0, rn), pl.ds(c0, cn))
        return hbm.at[sl], buf.at[sl], sem

    wq_cols = H * DH // WQ_C
    n_wq = (D_MODEL // WQ_R) * wq_cols

    def wq_piece(k):
        n = lax.rem(k * 11, jnp.int32(n_wq))
        r = lax.div(n, jnp.int32(wq_cols))
        c = n - wq_cols * r
        return piece(wq_hbm, wqbuf, wsem.at[0],
                     pl.multiple_of(r * WQ_R, WQ_R), WQ_R, pl.multiple_of(c * WQ_C, 128), WQ_C)

    wo_per_slice = GR // WO_R

    def wo_piece(k):
        gg = lax.div(k, jnp.int32(wo_per_slice))
        n = lax.rem((k - gg * wo_per_slice) * 7, jnp.int32(wo_per_slice))
        return piece(wo_hbm, wobuf, wsem.at[gg], pl.multiple_of(gg * GR + n * WO_R, WO_R), WO_R, 0, D_MODEL)

    def issue_wo(n):
        def f(i, carry):
            k = 2 * (n * WO_PER_STEP + i)
            start_pair(wo_piece(k), wo_piece(k + 1))
            return carry
        lax.fori_loop(0, WO_PER_STEP, f, 0, unroll=4)

    def ffn_sem(j):
        return kvsem.at[j // NQ, j % NQ]

    gu_lo = [sum(GU_GROUPS[:i]) for i in range(len(GU_GROUPS))]
    wd_lo = [sum(WD_GROUPS[:i]) for i in range(len(WD_GROUPS))]
    tail = []
    for i, n in enumerate(GU_GROUPS):
        for k in range(n // GU_R):
            tail.append(piece(wg_hbm, wgbuf, ffn_sem(i), gu_lo[i] + k * GU_R, GU_R, 0, FF))
            tail.append(piece(wu_hbm, wubuf, ffn_sem(i), gu_lo[i] + k * GU_R, GU_R, 0, FF))
    for i, n in enumerate(WD_GROUPS):
        for k in _scattered(n // WO_R, 7 if (n // WO_R) % 5 == 0 else 5):
            tail.append(piece(wd_hbm, wdbuf, ffn_sem(len(GU_GROUPS) + i), wd_lo[i] + k * WO_R, WO_R, 0, D_MODEL))
    tail_pos = [0]

    def issue_tail(n):
        lo = tail_pos[0]
        hi = min(lo + 2 * n, len(tail))
        for k in range(lo, hi, 2):
            start_pair(tail[k], tail[k + 1])
        tail_pos[0] = hi

    cx = pltpu.make_async_copy(x_hbm, xbuf, wsem.at[0])
    cwr = pltpu.make_async_copy(wr_hbm, wrbuf, wsem.at[0])

    row8 = lax.broadcasted_iota(jnp.int32, (8, GR), 0)
    lane8 = lax.broadcasted_iota(jnp.int32, (8, GR), 1)
    bd_mask = (lane8 >= row8 * DH) & (lane8 < (row8 + 1) * DH)

    cx.start(priority=TB)
    cwr.start(priority=TA)

    def first_wq(i, carry):
        start_pair(wq_piece(2 * i), wq_piece(2 * i + 1))
        return carry
    lax.fori_loop(0, n_wq // 2, first_wq, 0, unroll=4)
    issue_pass(0, 0)
    m_scr[...] = jnp.full(m_scr.shape, -jnp.inf, F32)
    l_scr[...] = jnp.zeros(l_scr.shape, F32)
    o_scr[...] = jnp.zeros(o_scr.shape, F32)
    cx.wait()
    cwr.wait()
    wait((wq_hbm, wqbuf, wsem.at[0]))
    ln1 = _ln(xbuf[...].astype(F32)).astype(BF16)

    def q_proj(gg, carry):
        cols = pl.ds(pl.multiple_of(gg * GR, 128), GR)
        q = jnp.dot(ln1, wqbuf[:, cols], preferred_element_type=F32)
        for b in range(B):
            qb = jnp.broadcast_to(q[b:b + 1, :], (8, GR))
            qbd_scr[b * GPB + gg] = jnp.where(bd_mask, qb, 0.0).astype(BF16)

        @pl.when(jnp.bitwise_and(gg, 1) == 1)
        def _():
            issue_kv(0, 1, lax.shift_right_logical(gg, 1))
        return carry
    lax.fori_loop(0, GPB, q_proj, 0)
    issue_pass(0, 2)
    issue_pass(0, 3)
    issue_pass(1, 0)

    def step(c, g):
        slot = lax.rem(c, jnp.int32(NR))
        rows = pl.ds(g * GA, GA)
        s = jnp.dot(qbd_scr[g], kbuf[slot, rows].reshape(GR, CW), preferred_element_type=F32)
        m_old = m_scr[g]
        m_new = jnp.maximum(m_old, jnp.broadcast_to(jnp.max(s, axis=1, keepdims=True), (8, CW)))
        alpha = jnp.exp((m_old - m_new) * SCALE)
        p = jnp.exp((s - m_new) * SCALE)
        m_scr[g] = m_new
        l_scr[g] = l_scr[g] * alpha + p
        pv = lax.dot_general(p.astype(BF16), vbuf[slot, rows].reshape(GR, CW), (((1,), (1,)), ((), ())),
                             preferred_element_type=F32)
        o_scr[g] = o_scr[g] * alpha[:, 0:1] + pv

    def super_step(n, carry):
        c = lax.shift_right_logical(n, 3)
        i = jnp.bitwise_and(n, NSS - 1)

        @pl.when(jnp.bitwise_and(i, NSS // NQ - 1) == 0)
        def _():
            q = lax.div(i, jnp.int32(NSS // NQ))
            wait(kv_part(k_hbm, kbuf, c, q))
            wait(kv_part(v_hbm, vbuf, c, q))
        step(c, 2 * i)
        step(c, 2 * i + 1)

        m = n + AHEAD
        cm = lax.shift_right_logical(m, 3)
        sm = jnp.bitwise_and(lax.shift_right_logical(m, 1), NS - 1)
        par = jnp.bitwise_and(m, 1)
        for s in range(NS):
            @pl.when((sm == s) & (cm < NC))
            def _():
                issue_kv(cm, s, par)

        nw = m - NC * NSS

        @pl.when((nw >= 0) & (nw < GPB * wo_per_slice // (2 * WO_PER_STEP)))
        def _():
            issue_wo(nw)
        return carry

    lax.fori_loop(0, NC * NSS, super_step, 0)

    attn = jnp.zeros((8, D_MODEL), F32)
    for gg in range(GPB):
        issue_tail(TAIL_PER_SLICE[gg])
        oin = jnp.zeros((8, GR), F32)
        for b in range(B):
            g = b * GPB + gg
            l = jnp.sum(l_scr[g], axis=1, keepdims=True)
            o = jnp.where(bd_mask, o_scr[g] / l, 0.0)
            orow = jnp.sum(o, axis=0, keepdims=True)
            oin = jnp.where(row8 == b, jnp.broadcast_to(orow, (8, GR)), oin)
        sl = pl.ds(gg * GR, GR)
        wait((wo_hbm.at[sl], wobuf.at[sl], wsem.at[gg]))
        attn = attn + jnp.dot(oin.astype(BF16), wobuf[sl, :], preferred_element_type=F32)

    h = xbuf[...].astype(F32) + attn[0:B, :]
    ln2 = _ln(h)
    ln2b = ln2.astype(BF16)
    r = jnp.sum(ln2b.astype(F32) * wrbuf[...].astype(F32)[None, :], axis=1, keepdims=True)
    issue_tail(len(tail))
    gt = jnp.zeros((B, FF), F32)
    up = jnp.zeros((B, FF), F32)
    for i, n in enumerate(GU_GROUPS):
        sl = pl.ds(gu_lo[i], n)
        wait((wg_hbm.at[sl], wgbuf.at[sl], ffn_sem(i)))
        wait((wu_hbm.at[sl], wubuf.at[sl], ffn_sem(i)))
        lhs = ln2b[:, gu_lo[i]:gu_lo[i] + n]
        gt = gt + jnp.dot(lhs, wgbuf[sl, :], preferred_element_type=F32)
        up = up + jnp.dot(lhs, wubuf[sl, :], preferred_element_type=F32)
    act = (gt * jax.nn.sigmoid(gt) * up).astype(BF16)
    y = jnp.zeros((B, D_MODEL), F32)
    for i, n in enumerate(WD_GROUPS):
        sl = pl.ds(wd_lo[i], n)
        wait((wd_hbm.at[sl], wdbuf.at[sl], ffn_sem(len(GU_GROUPS) + i)))
        y = y + jnp.dot(act[:, wd_lo[i]:wd_lo[i] + n], wdbuf[sl, :], preferred_element_type=F32)
    out = h + (ln2 + y * jax.nn.sigmoid(r))
    out_ref[...] = out.astype(out_ref.dtype)


@jax.jit
def pallas_sequential_preLN__mha_block_cached__moe_arch_mod__decode_kernel(
    A_x, A_k_cache, A_v_cache, A_wq, A_wo, B_x, B_w_r, B_w_gate, B_w_up, B_w_down
):
    del B_x
    kt = jnp.swapaxes(A_k_cache, 2, 3).reshape(NA, 2, 8, SK)
    vt = jnp.swapaxes(A_v_cache, 2, 3).reshape(NA, 2, 8, SK)
    x2 = A_x.reshape(B, D_MODEL)
    anyspec = pl.BlockSpec(memory_space=pl.ANY)
    ring = pltpu.VMEM((NR, NA, 2, 8, CW), BF16)
    out = pl.pallas_call(
        _kernel,
        in_specs=[anyspec] * 9,
        out_specs=pl.BlockSpec(memory_space=pltpu.VMEM),
        out_shape=jax.ShapeDtypeStruct((B, D_MODEL), BF16),
        scratch_shapes=[
            pltpu.VMEM((B, D_MODEL), BF16),
            pltpu.VMEM((D_MODEL,), BF16),
            pltpu.VMEM((D_MODEL, H * DH), BF16),
            pltpu.VMEM((H * DH, D_MODEL), BF16),
            pltpu.VMEM((D_MODEL, FF), BF16),
            pltpu.VMEM((D_MODEL, FF), BF16),
            pltpu.VMEM((FF, D_MODEL), BF16),
            ring, ring,
            pltpu.VMEM((NG, 8, GR), BF16),
            pltpu.VMEM((NG, 8, CW), F32),
            pltpu.VMEM((NG, 8, CW), F32),
            pltpu.VMEM((NG, 8, GR), F32),
            pltpu.SemaphoreType.DMA((NR, NQ)),
            pltpu.SemaphoreType.DMA((GPB,)),
        ],
        compiler_params=pltpu.CompilerParams(vmem_limit_bytes=100 * 1024 * 1024),
    )(x2, kt, vt, A_wq, A_wo, B_w_r, B_w_gate, B_w_up, B_w_down)
    return out.reshape(B, 1, D_MODEL)
```

```python
import jax
import jax.numpy as jnp
from jax import lax
from jax.experimental import pallas as pl
from jax.experimental.pallas import tpu as pltpu

B, D_MODEL, H, SK, DH, FF = 4, 640, 32, 8192, 192, 1536
CW = 128
NC = SK // CW
NA = B * H * DH // 16
HG = 8
GR = HG * DH
GA = GR // 16
NG = NA // GA
GPB = H // HG
RT = 64
NS = 4
NAB = NA // RT
NR = 3
NQ = 2
NSS = NG // 2
AHEAD = NSS + 2
WQ_R, WQ_C = 8, 2048
WO_R = 32
GU_R = 16
WO_PER_STEP = 16
GU_GROUPS = (256, 256, 128)
WD_GROUPS = (512, 512, 512)
TAIL_PER_SLICE = (24, 12, 12, 12)
TA, TB = 1, 0
EPS = 1e-5
SCALE = DH ** -0.5
F32 = jnp.float32
BF16 = jnp.bfloat16


def _ln(x):
    m = jnp.mean(x, axis=-1, keepdims=True)
    xc = x - m
    v = jnp.mean(xc * xc, axis=-1, keepdims=True)
    return xc * lax.rsqrt(v + EPS)


def _scattered(n, m):
    return [(k * m) % n for k in range(n)]


def _kernel(x_hbm, k_hbm, v_hbm, wq_hbm, wo_hbm, wr_hbm, wg_hbm, wu_hbm, wd_hbm, out_ref,
            xbuf, wrbuf, wqbuf, wobuf, wgbuf, wubuf, wdbuf, kbuf, vbuf, qbd_scr, m_scr, l_scr, o_scr,
            kvsem, wsem):

    def start_pair(a, b):
        for (src, dst, sem), prio in ((a, TA), (b, TB)):
            pltpu.make_async_copy(src, dst, sem).start(priority=prio)

    def wait(d):
        pltpu.make_async_copy(*d).wait()

    def col_slice(c):
        return pl.ds(pl.multiple_of(c * CW, CW), CW)

    caches = ((k_hbm, kbuf), (v_hbm, vbuf))

    def issue_kv(c, s, h):
        slot = lax.rem(c, jnp.int32(NR))
        col = col_slice(c)
        sub = pl.ds(s * 2, 2)
        for hbm, buf in caches:
            for ab in range(h * NAB // 2, (h + 1) * NAB // 2):
                rows = pl.ds(ab * RT, RT)
                sem = kvsem.at[slot, ab // (NAB // NQ)]
                start_pair((hbm.at[rows, 0, sub, col], buf.at[slot, rows, 0, sub], sem),
                           (hbm.at[rows, 1, sub, col], buf.at[slot, rows, 1, sub], sem))

    def issue_half_pass(m):
        c = lax.shift_right_logical(m, 3)
        sm = jnp.bitwise_and(lax.shift_right_logical(m, 1), NS - 1)
        hm = jnp.bitwise_and(m, 1)
        for s in range(NS):
            for h in range(2):
                @pl.when((sm == s) & (hm == h) & (c < NC))
                def _():
                    issue_kv(c, s, h)

    def kv_part(hbm, buf, c, q):
        slot = lax.rem(c, jnp.int32(NR))
        rows = pl.ds(q * (NA // NQ), NA // NQ)
        return hbm.at[rows, :, :, col_slice(c)], buf.at[slot, rows], kvsem.at[slot, q]

    def piece(hbm, buf, sem, r0, rn, c0, cn):
        sl = (pl.ds(r0, rn), pl.ds(c0, cn))
        return hbm.at[sl], buf.at[sl], sem

    wq_cols = H * DH // WQ_C
    n_wq = (D_MODEL // WQ_R) * wq_cols

    def wq_piece(k):
        n = lax.rem(k * 11, jnp.int32(n_wq))
        r = lax.div(n, jnp.int32(wq_cols))
        c = n - wq_cols * r
        return piece(wq_hbm, wqbuf, wsem.at[0],
                     pl.multiple_of(r * WQ_R, WQ_R), WQ_R, pl.multiple_of(c * WQ_C, 128), WQ_C)

    wo_per_slice = GR // WO_R

    def wo_piece(k):
        gg = lax.div(k, jnp.int32(wo_per_slice))
        n = lax.rem((k - gg * wo_per_slice) * 7, jnp.int32(wo_per_slice))
        return piece(wo_hbm, wobuf, wsem.at[gg], pl.multiple_of(gg * GR + n * WO_R, WO_R), WO_R, 0, D_MODEL)

    def issue_wo(n):
        def f(i, carry):
            k = 2 * (n * WO_PER_STEP + i)
            start_pair(wo_piece(k), wo_piece(k + 1))
            return carry
        lax.fori_loop(0, WO_PER_STEP, f, 0, unroll=4)

    def ffn_sem(j):
        return kvsem.at[j // NQ, j % NQ]

    gu_lo = [sum(GU_GROUPS[:i]) for i in range(len(GU_GROUPS))]
    wd_lo = [sum(WD_GROUPS[:i]) for i in range(len(WD_GROUPS))]
    tail = []
    for i, n in enumerate(GU_GROUPS):
        for k in range(n // GU_R):
            tail.append(piece(wg_hbm, wgbuf, ffn_sem(i), gu_lo[i] + k * GU_R, GU_R, 0, FF))
            tail.append(piece(wu_hbm, wubuf, ffn_sem(i), gu_lo[i] + k * GU_R, GU_R, 0, FF))
    for i, n in enumerate(WD_GROUPS):
        for k in _scattered(n // WO_R, 7 if (n // WO_R) % 5 == 0 else 5):
            tail.append(piece(wd_hbm, wdbuf, ffn_sem(len(GU_GROUPS) + i), wd_lo[i] + k * WO_R, WO_R, 0, D_MODEL))
    tail_pos = [0]

    def issue_tail(n):
        lo = tail_pos[0]
        hi = min(lo + 2 * n, len(tail))
        for k in range(lo, hi, 2):
            start_pair(tail[k], tail[k + 1])
        tail_pos[0] = hi

    cx = pltpu.make_async_copy(x_hbm, xbuf, wsem.at[0])
    cwr = pltpu.make_async_copy(wr_hbm, wrbuf, wsem.at[0])

    row8 = lax.broadcasted_iota(jnp.int32, (8, GR), 0)
    lane8 = lax.broadcasted_iota(jnp.int32, (8, GR), 1)
    bd_mask = (lane8 >= row8 * DH) & (lane8 < (row8 + 1) * DH)

    cx.start(priority=TB)
    cwr.start(priority=TA)

    def first_wq(i, carry):
        start_pair(wq_piece(2 * i), wq_piece(2 * i + 1))
        return carry
    lax.fori_loop(0, n_wq // 2, first_wq, 0, unroll=4)
    issue_kv(0, 0, 0)
    issue_kv(0, 0, 1)
    m_scr[...] = jnp.full(m_scr.shape, -jnp.inf, F32)
    l_scr[...] = jnp.zeros(l_scr.shape, F32)
    o_scr[...] = jnp.zeros(o_scr.shape, F32)
    cx.wait()
    cwr.wait()
    wait((wq_hbm, wqbuf, wsem.at[0]))
    ln1 = _ln(xbuf[...].astype(F32)).astype(BF16)

    def q_proj(gg, carry):
        cols = pl.ds(pl.multiple_of(gg * GR, 128), GR)
        q = jnp.dot(ln1, wqbuf[:, cols], preferred_element_type=F32)
        for b in range(B):
            qb = jnp.broadcast_to(q[b:b + 1, :], (8, GR))
            qbd_scr[b * GPB + gg] = jnp.where(bd_mask, qb, 0.0).astype(BF16)

        @pl.when(jnp.bitwise_and(gg, 1) == 1)
        def _():
            issue_half_pass(2 + lax.shift_right_logical(gg, 1))
        return carry
    lax.fori_loop(0, GPB, q_proj, 0)

    def rest(m, carry):
        issue_half_pass(m)
        return carry
    lax.fori_loop(4, AHEAD, rest, 0)

    def step(c, g):
        slot = lax.rem(c, jnp.int32(NR))
        rows = pl.ds(g * GA, GA)
        s = jnp.dot(qbd_scr[g], kbuf[slot, rows].reshape(GR, CW), preferred_element_type=F32)
        m_old = m_scr[g]
        m_new = jnp.maximum(m_old, jnp.broadcast_to(jnp.max(s, axis=1, keepdims=True), (8, CW)))
        alpha = jnp.exp((m_old - m_new) * SCALE)
        p = jnp.exp((s - m_new) * SCALE)
        m_scr[g] = m_new
        l_scr[g] = l_scr[g] * alpha + p
        pv = lax.dot_general(p.astype(BF16), vbuf[slot, rows].reshape(GR, CW), (((1,), (1,)), ((), ())),
                             preferred_element_type=F32)
        o_scr[g] = o_scr[g] * alpha[:, 0:1] + pv

    def super_step(n, carry):
        c = lax.shift_right_logical(n, 3)
        i = jnp.bitwise_and(n, NSS - 1)

        @pl.when(jnp.bitwise_and(i, NSS // NQ - 1) == 0)
        def _():
            q = lax.div(i, jnp.int32(NSS // NQ))
            wait(kv_part(k_hbm, kbuf, c, q))
            wait(kv_part(v_hbm, vbuf, c, q))
        step(c, 2 * i)
        step(c, 2 * i + 1)

        m = n + AHEAD
        issue_half_pass(m)
        nw = m - NC * NSS

        @pl.when((nw >= 0) & (nw < GPB * wo_per_slice // (2 * WO_PER_STEP)))
        def _():
            issue_wo(nw)
        return carry

    lax.fori_loop(0, NC * NSS, super_step, 0)

    attn = jnp.zeros((8, D_MODEL), F32)
    for gg in range(GPB):
        issue_tail(TAIL_PER_SLICE[gg])
        oin = jnp.zeros((8, GR), F32)
        for b in range(B):
            g = b * GPB + gg
            l = jnp.sum(l_scr[g], axis=1, keepdims=True)
            o = jnp.where(bd_mask, o_scr[g] / l, 0.0)
            orow = jnp.sum(o, axis=0, keepdims=True)
            oin = jnp.where(row8 == b, jnp.broadcast_to(orow, (8, GR)), oin)
        sl = pl.ds(gg * GR, GR)
        wait((wo_hbm.at[sl], wobuf.at[sl], wsem.at[gg]))
        attn = attn + jnp.dot(oin.astype(BF16), wobuf[sl, :], preferred_element_type=F32)

    h = xbuf[...].astype(F32) + attn[0:B, :]
    ln2 = _ln(h)
    ln2b = ln2.astype(BF16)
    r = jnp.sum(ln2b.astype(F32) * wrbuf[...].astype(F32)[None, :], axis=1, keepdims=True)
    issue_tail(len(tail))
    gt = jnp.zeros((B, FF), F32)
    up = jnp.zeros((B, FF), F32)
    for i, n in enumerate(GU_GROUPS):
        sl = pl.ds(gu_lo[i], n)
        wait((wg_hbm.at[sl], wgbuf.at[sl], ffn_sem(i)))
        wait((wu_hbm.at[sl], wubuf.at[sl], ffn_sem(i)))
        lhs = ln2b[:, gu_lo[i]:gu_lo[i] + n]
        gt = gt + jnp.dot(lhs, wgbuf[sl, :], preferred_element_type=F32)
        up = up + jnp.dot(lhs, wubuf[sl, :], preferred_element_type=F32)
    act = (gt * jax.nn.sigmoid(gt) * up).astype(BF16)
    y = jnp.zeros((B, D_MODEL), F32)
    for i, n in enumerate(WD_GROUPS):
        sl = pl.ds(wd_lo[i], n)
        wait((wd_hbm.at[sl], wdbuf.at[sl], ffn_sem(len(GU_GROUPS) + i)))
        y = y + jnp.dot(act[:, wd_lo[i]:wd_lo[i] + n], wdbuf[sl, :], preferred_element_type=F32)
    out = h + (ln2 + y * jax.nn.sigmoid(r))
    out_ref[...] = out.astype(out_ref.dtype)


@jax.jit
def pallas_sequential_preLN__mha_block_cached__moe_arch_mod__decode_kernel(
    A_x, A_k_cache, A_v_cache, A_wq, A_wo, B_x, B_w_r, B_w_gate, B_w_up, B_w_down
):
    del B_x
    kt = jnp.swapaxes(A_k_cache, 2, 3).reshape(NA, 2, 8, SK)
    vt = jnp.swapaxes(A_v_cache, 2, 3).reshape(NA, 2, 8, SK)
    x2 = A_x.reshape(B, D_MODEL)
    anyspec = pl.BlockSpec(memory_space=pl.ANY)
    ring = pltpu.VMEM((NR, NA, 2, 8, CW), BF16)
    out = pl.pallas_call(
        _kernel,
        in_specs=[anyspec] * 9,
        out_specs=pl.BlockSpec(memory_space=pltpu.VMEM),
        out_shape=jax.ShapeDtypeStruct((B, D_MODEL), BF16),
        scratch_shapes=[
            pltpu.VMEM((B, D_MODEL), BF16),
            pltpu.VMEM((D_MODEL,), BF16),
            pltpu.VMEM((D_MODEL, H * DH), BF16),
            pltpu.VMEM((H * DH, D_MODEL), BF16),
            pltpu.VMEM((D_MODEL, FF), BF16),
            pltpu.VMEM((D_MODEL, FF), BF16),
            pltpu.VMEM((FF, D_MODEL), BF16),
            ring, ring,
            pltpu.VMEM((NG, 8, GR), BF16),
            pltpu.VMEM((NG, 8, CW), F32),
            pltpu.VMEM((NG, 8, CW), F32),
            pltpu.VMEM((NG, 8, GR), F32),
            pltpu.SemaphoreType.DMA((NR, NQ)),
            pltpu.SemaphoreType.DMA((GPB,)),
        ],
        compiler_params=pltpu.CompilerParams(vmem_limit_bytes=100 * 1024 * 1024),
    )(x2, kt, vt, A_wq, A_wo, B_w_r, B_w_gate, B_w_up, B_w_down)
    return out.reshape(B, 1, D_MODEL)
```

```python
import jax
import jax.numpy as jnp
from jax import lax
from jax.experimental import pallas as pl
from jax.experimental.pallas import tpu as pltpu

B, D_MODEL, H, SK, DH, FF = 4, 640, 32, 8192, 192, 1536
CW = 128
NC = SK // CW
NA = B * H * DH // 16
HG = 8
GR = HG * DH
GA = GR // 16
NG = NA // GA
GPB = H // HG
RT = 64
NHP = 8
NAB = NA // RT
NR = 3
NQ = 2
NSS = NG // 2
AHEAD = NHP + 2
WQ_R, WQ_C = 8, 2048
WO_R = 32
GU_R = 16
WO_PER_STEP = 14
GU_GROUPS = (256, 256, 128)
WD_GROUPS = (512, 512, 512)
TAIL_PER_SLICE = (24, 12, 12, 12)
TA, TB = 0, 1
SKEW = 26
EPS = 1e-5
SCALE = DH ** -0.5
F32 = jnp.float32
BF16 = jnp.bfloat16


def _ln(x):
    m = jnp.mean(x, axis=-1, keepdims=True)
    xc = x - m
    v = jnp.mean(xc * xc, axis=-1, keepdims=True)
    return xc * lax.rsqrt(v + EPS)


def _scattered(n, m):
    return [(k * m) % n for k in range(n)]


def _kernel(x_hbm, k_hbm, v_hbm, wq_hbm, wo_hbm, wr_hbm, wg_hbm, wu_hbm, wd_hbm, out_ref,
            xbuf, wrbuf, wqbuf, wobuf, wgbuf, wubuf, wdbuf, kbuf, vbuf, qbd_scr, m_scr, l_scr, o_scr,
            kvsem, wsem):

    def start_pair(a, b):
        for (src, dst, sem), prio in ((a, TA), (b, TB)):
            pltpu.make_async_copy(src, dst, sem).start(priority=prio)

    def wait(d):
        pltpu.make_async_copy(*d).wait()

    def col_slice(c):
        return pl.ds(pl.multiple_of(c * CW, CW), CW)

    caches = ((k_hbm, kbuf), (v_hbm, vbuf))

    def kv_copy(c, hp, j, par):
        dc, pos = divmod(hp * NAB + j, NHP * NAB)
        hp2, ab = divmod(pos, NAB)
        s, x = divmod(hp2, 2)
        hbm, buf = caches[x]
        slot = lax.rem(c + dc, jnp.int32(NR))
        rows = pl.ds(ab * RT, RT)
        sub = pl.ds(s * 2, 2)
        return (hbm.at[rows, par, sub, col_slice(c + dc)], buf.at[slot, rows, par, sub],
                kvsem.at[slot, ab // (NAB // NQ)])

    def issue_kv(c, hp, ending=False):
        for j in range(NAB):
            over = hp * NAB + j + SKEW - NHP * NAB
            b = wo_piece(over) if ending and over >= 0 else kv_copy(c, hp, j + SKEW, 1)
            start_pair(kv_copy(c, hp, j, 0), b)

    def issue_half_pass(m):
        c = lax.shift_right_logical(m, 3)
        hm = jnp.bitwise_and(m, NHP - 1)
        for hp in range(NHP):
            if (hp + 1) * NAB - 1 + SKEW >= NHP * NAB:
                @pl.when((hm == hp) & (c < NC - 1))
                def _():
                    issue_kv(c, hp)

                @pl.when((hm == hp) & (c == NC - 1))
                def _():
                    issue_kv(c, hp, ending=True)
            else:
                @pl.when((hm == hp) & (c < NC))
                def _():
                    issue_kv(c, hp)

    def kv_part(hbm, buf, c, q):
        slot = lax.rem(c, jnp.int32(NR))
        rows = pl.ds(q * (NA // NQ), NA // NQ)
        return hbm.at[rows, :, :, col_slice(c)], buf.at[slot, rows], kvsem.at[slot, q]

    def piece(hbm, buf, sem, r0, rn, c0, cn):
        sl = (pl.ds(r0, rn), pl.ds(c0, cn))
        return hbm.at[sl], buf.at[sl], sem

    wq_cols = H * DH // WQ_C
    n_wq = (D_MODEL // WQ_R) * wq_cols

    def wq_piece(k):
        n = lax.rem(k * 11, jnp.int32(n_wq))
        r = lax.div(n, jnp.int32(wq_cols))
        c = n - wq_cols * r
        return piece(wq_hbm, wqbuf, wsem.at[0],
                     pl.multiple_of(r * WQ_R, WQ_R), WQ_R, pl.multiple_of(c * WQ_C, 128), WQ_C)

    wo_per_slice = GR // WO_R

    def wo_piece(k):
        k = jnp.asarray(k, jnp.int32)
        gg = lax.div(k, jnp.int32(wo_per_slice))
        n = lax.rem((k - gg * wo_per_slice) * 7, jnp.int32(wo_per_slice))
        return piece(wo_hbm, wobuf, wsem.at[gg], pl.multiple_of(gg * GR + n * WO_R, WO_R), WO_R, 0, D_MODEL)

    def issue_wo(n):
        def f(i, carry):
            k = SKEW + 2 * (n * WO_PER_STEP + i)

            @pl.when(k < GPB * wo_per_slice)
            def _():
                start_pair(wo_piece(k), wo_piece(k + 1))
            return carry
        lax.fori_loop(0, WO_PER_STEP, f, 0, unroll=4)

    def ffn_sem(j):
        return kvsem.at[j // NQ, j % NQ]

    gu_lo = [sum(GU_GROUPS[:i]) for i in range(len(GU_GROUPS))]
    wd_lo = [sum(WD_GROUPS[:i]) for i in range(len(WD_GROUPS))]
    tail = []
    for i, n in enumerate(GU_GROUPS):
        for k in range(n // GU_R):
            tail.append(piece(wg_hbm, wgbuf, ffn_sem(i), gu_lo[i] + k * GU_R, GU_R, 0, FF))
            tail.append(piece(wu_hbm, wubuf, ffn_sem(i), gu_lo[i] + k * GU_R, GU_R, 0, FF))
    for i, n in enumerate(WD_GROUPS):
        for k in _scattered(n // WO_R, 7 if (n // WO_R) % 5 == 0 else 5):
            tail.append(piece(wd_hbm, wdbuf, ffn_sem(len(GU_GROUPS) + i), wd_lo[i] + k * WO_R, WO_R, 0, D_MODEL))
    tail_pos = [0]

    def issue_tail(n):
        lo = tail_pos[0]
        hi = min(lo + 2 * n, len(tail))
        for k in range(lo, hi, 2):
            start_pair(tail[k], tail[k + 1])
        tail_pos[0] = hi

    cx = pltpu.make_async_copy(x_hbm, xbuf, wsem.at[0])
    cwr = pltpu.make_async_copy(wr_hbm, wrbuf, wsem.at[0])

    row8 = lax.broadcasted_iota(jnp.int32, (8, GR), 0)
    lane8 = lax.broadcasted_iota(jnp.int32, (8, GR), 1)
    bd_mask = (lane8 >= row8 * DH) & (lane8 < (row8 + 1) * DH)

    cx.start(priority=TB)
    cwr.start(priority=TA)
    for j in range(SKEW):
        pltpu.make_async_copy(*kv_copy(0, 0, j, 1)).start(priority=TB)

    def first_wq(i, carry):
        start_pair(wq_piece(2 * i), wq_piece(2 * i + 1))
        return carry
    lax.fori_loop(0, n_wq // 2, first_wq, 0, unroll=4)
    issue_kv(0, 0)
    issue_kv(0, 1)
    m_scr[...] = jnp.full(m_scr.shape, -jnp.inf, F32)
    l_scr[...] = jnp.zeros(l_scr.shape, F32)
    o_scr[...] = jnp.zeros(o_scr.shape, F32)
    cx.wait()
    cwr.wait()
    wait((wq_hbm, wqbuf, wsem.at[0]))
    ln1 = _ln(xbuf[...].astype(F32)).astype(BF16)

    def q_proj(gg, carry):
        cols = pl.ds(pl.multiple_of(gg * GR, 128), GR)
        q = jnp.dot(ln1, wqbuf[:, cols], preferred_element_type=F32)
        for b in range(B):
            qb = jnp.broadcast_to(q[b:b + 1, :], (8, GR))
            qbd_scr[b * GPB + gg] = jnp.where(bd_mask, qb, 0.0).astype(BF16)

        @pl.when(jnp.bitwise_and(gg, 1) == 1)
        def _():
            issue_half_pass(2 + lax.shift_right_logical(gg, 1))
        return carry
    lax.fori_loop(0, GPB, q_proj, 0)

    def rest(m, carry):
        issue_half_pass(m)
        return carry
    lax.fori_loop(4, AHEAD, rest, 0)

    def step(c, g):
        slot = lax.rem(c, jnp.int32(NR))
        rows = pl.ds(g * GA, GA)
        s = jnp.dot(qbd_scr[g], kbuf[slot, rows].reshape(GR, CW), preferred_element_type=F32)
        m_old = m_scr[g]
        m_new = jnp.maximum(m_old, jnp.broadcast_to(jnp.max(s, axis=1, keepdims=True), (8, CW)))
        alpha = jnp.exp((m_old - m_new) * SCALE)
        p = jnp.exp((s - m_new) * SCALE)
        m_scr[g] = m_new
        l_scr[g] = l_scr[g] * alpha + p
        pv = lax.dot_general(p.astype(BF16), vbuf[slot, rows].reshape(GR, CW), (((1,), (1,)), ((), ())),
                             preferred_element_type=F32)
        o_scr[g] = o_scr[g] * alpha[:, 0:1] + pv

    def super_step(n, carry):
        c = lax.shift_right_logical(n, 3)
        i = jnp.bitwise_and(n, NSS - 1)

        @pl.when(jnp.bitwise_and(i, NSS // NQ - 1) == 0)
        def _():
            q = lax.div(i, jnp.int32(NSS // NQ))
            wait(kv_part(k_hbm, kbuf, c, q))
            wait(kv_part(v_hbm, vbuf, c, q))
        step(c, 2 * i)
        step(c, 2 * i + 1)

        m = n + AHEAD
        issue_half_pass(m)
        nw = m - NC * NSS

        @pl.when((nw >= 0) & (nw < -(-(GPB * wo_per_slice - SKEW) // (2 * WO_PER_STEP))))
        def _():
            issue_wo(nw)
        return carry

    lax.fori_loop(0, NC * NSS, super_step, 0)

    attn = jnp.zeros((8, D_MODEL), F32)
    for gg in range(GPB):
        issue_tail(TAIL_PER_SLICE[gg])
        oin = jnp.zeros((8, GR), F32)
        for b in range(B):
            g = b * GPB + gg
            l = jnp.sum(l_scr[g], axis=1, keepdims=True)
            o = jnp.where(bd_mask, o_scr[g] / l, 0.0)
            orow = jnp.sum(o, axis=0, keepdims=True)
            oin = jnp.where(row8 == b, jnp.broadcast_to(orow, (8, GR)), oin)
        sl = pl.ds(gg * GR, GR)
        wait((wo_hbm.at[sl], wobuf.at[sl], wsem.at[gg]))
        attn = attn + jnp.dot(oin.astype(BF16), wobuf[sl, :], preferred_element_type=F32)

    h = xbuf[...].astype(F32) + attn[0:B, :]
    ln2 = _ln(h)
    ln2b = ln2.astype(BF16)
    r = jnp.sum(ln2b.astype(F32) * wrbuf[...].astype(F32)[None, :], axis=1, keepdims=True)
    issue_tail(len(tail))
    gt = jnp.zeros((B, FF), F32)
    up = jnp.zeros((B, FF), F32)
    for i, n in enumerate(GU_GROUPS):
        sl = pl.ds(gu_lo[i], n)
        wait((wg_hbm.at[sl], wgbuf.at[sl], ffn_sem(i)))
        wait((wu_hbm.at[sl], wubuf.at[sl], ffn_sem(i)))
        lhs = ln2b[:, gu_lo[i]:gu_lo[i] + n]
        gt = gt + jnp.dot(lhs, wgbuf[sl, :], preferred_element_type=F32)
        up = up + jnp.dot(lhs, wubuf[sl, :], preferred_element_type=F32)
    act = (gt * jax.nn.sigmoid(gt) * up).astype(BF16)
    y = jnp.zeros((B, D_MODEL), F32)
    for i, n in enumerate(WD_GROUPS):
        sl = pl.ds(wd_lo[i], n)
        wait((wd_hbm.at[sl], wdbuf.at[sl], ffn_sem(len(GU_GROUPS) + i)))
        y = y + jnp.dot(act[:, wd_lo[i]:wd_lo[i] + n], wdbuf[sl, :], preferred_element_type=F32)
    out = h + (ln2 + y * jax.nn.sigmoid(r))
    out_ref[...] = out.astype(out_ref.dtype)


@jax.jit
def pallas_sequential_preLN__mha_block_cached__moe_arch_mod__decode_kernel(
    A_x, A_k_cache, A_v_cache, A_wq, A_wo, B_x, B_w_r, B_w_gate, B_w_up, B_w_down
):
    del B_x
    kt = jnp.swapaxes(A_k_cache, 2, 3).reshape(NA, 2, 8, SK)
    vt = jnp.swapaxes(A_v_cache, 2, 3).reshape(NA, 2, 8, SK)
    x2 = A_x.reshape(B, D_MODEL)
    anyspec = pl.BlockSpec(memory_space=pl.ANY)
    ring = pltpu.VMEM((NR, NA, 2, 8, CW), BF16)
    out = pl.pallas_call(
        _kernel,
        in_specs=[anyspec] * 9,
        out_specs=pl.BlockSpec(memory_space=pltpu.VMEM),
        out_shape=jax.ShapeDtypeStruct((B, D_MODEL), BF16),
        scratch_shapes=[
            pltpu.VMEM((B, D_MODEL), BF16),
            pltpu.VMEM((D_MODEL,), BF16),
            pltpu.VMEM((D_MODEL, H * DH), BF16),
            pltpu.VMEM((H * DH, D_MODEL), BF16),
            pltpu.VMEM((D_MODEL, FF), BF16),
            pltpu.VMEM((D_MODEL, FF), BF16),
            pltpu.VMEM((FF, D_MODEL), BF16),
            ring, ring,
            pltpu.VMEM((NG, 8, GR), BF16),
            pltpu.VMEM((NG, 8, CW), F32),
            pltpu.VMEM((NG, 8, CW), F32),
            pltpu.VMEM((NG, 8, GR), F32),
            pltpu.SemaphoreType.DMA((NR, NQ)),
            pltpu.SemaphoreType.DMA((GPB,)),
        ],
        compiler_params=pltpu.CompilerParams(vmem_limit_bytes=100 * 1024 * 1024),
    )(x2, kt, vt, A_wq, A_wo, B_w_r, B_w_gate, B_w_up, B_w_down)
    return out.reshape(B, 1, D_MODEL)
```

```python
import jax
import jax.numpy as jnp
from jax import lax
from jax.experimental import pallas as pl
from jax.experimental.pallas import tpu as pltpu

B, D_MODEL, H, SK, DH, FF = 4, 640, 32, 8192, 192, 1536
CW = 128
NC = SK // CW
NA = B * H * DH // 16
HG = 8
GR = HG * DH
GA = GR // 16
NG = NA // GA
GPB = H // HG
RT = 64
NHP = 8
NAB = NA // RT
NR = 3
NQ = 2
NSS = NG // 2
AHEAD = NHP + 2
WQ_R, WQ_C = 8, 2048
WO_R = 32
GU_R = 16
WO_PER_STEP = 14
GU_GROUPS = (256, 256, 128)
WD_GROUPS = (512, 512, 512)
TAIL_PER_SLICE = (24, 12, 12, 12)
TA, TB = 0, 1
SKEW = 26
EPS = 1e-5
SCALE = DH ** -0.5
F32 = jnp.float32
BF16 = jnp.bfloat16


def _ln(x):
    m = jnp.mean(x, axis=-1, keepdims=True)
    xc = x - m
    v = jnp.mean(xc * xc, axis=-1, keepdims=True)
    return xc * lax.rsqrt(v + EPS)


def _scattered(n, m):
    return [(k * m) % n for k in range(n)]


def _kernel(x_hbm, k_hbm, v_hbm, wq_hbm, wo_hbm, wr_hbm, wg_hbm, wu_hbm, wd_hbm, out_ref,
            xbuf, wrbuf, wqbuf, wobuf, wgbuf, wubuf, wdbuf, kbuf, vbuf, qbd_scr, m_scr, l_scr, o_scr,
            kvsem, wsem):

    def start_pair(a, b):
        for (src, dst, sem), prio in ((a, TA), (b, TB)):
            pltpu.make_async_copy(src, dst, sem).start(priority=prio)

    def wait(d):
        pltpu.make_async_copy(*d).wait()

    def col_slice(c):
        return pl.ds(pl.multiple_of(c * CW, CW), CW)

    caches = ((k_hbm, kbuf), (v_hbm, vbuf))

    def kv_copy(c, hp, j, odd):
        dc, pos = divmod(hp * NAB + j, NHP * NAB)
        hp2, i = divmod(pos, NAB)
        s, par = divmod(hp2, 2)
        x, i = divmod(i, NAB // 2)
        ab = 2 * i + odd
        hbm, buf = caches[x]
        slot = lax.rem(c + dc, jnp.int32(NR))
        rows = pl.ds(ab * RT, RT)
        sub = pl.ds(s * 2, 2)
        return (hbm.at[rows, par, sub, col_slice(c + dc)], buf.at[slot, rows, par, sub],
                kvsem.at[slot, ab // (NAB // NQ)])

    def issue_kv(c, hp, ending=False):
        for j in range(NAB):
            over = hp * NAB + j + SKEW - NHP * NAB
            b = wo_piece(over) if ending and over >= 0 else kv_copy(c, hp, j + SKEW, 1)
            start_pair(kv_copy(c, hp, j, 0), b)

    def issue_half_pass(m):
        c = lax.shift_right_logical(m, 3)
        hm = jnp.bitwise_and(m, NHP - 1)
        for hp in range(NHP):
            if (hp + 1) * NAB - 1 + SKEW >= NHP * NAB:
                @pl.when((hm == hp) & (c < NC - 1))
                def _():
                    issue_kv(c, hp)

                @pl.when((hm == hp) & (c == NC - 1))
                def _():
                    issue_kv(c, hp, ending=True)
            else:
                @pl.when((hm == hp) & (c < NC))
                def _():
                    issue_kv(c, hp)

    def kv_part(hbm, buf, c, q):
        slot = lax.rem(c, jnp.int32(NR))
        rows = pl.ds(q * (NA // NQ), NA // NQ)
        return hbm.at[rows, :, :, col_slice(c)], buf.at[slot, rows], kvsem.at[slot, q]

    def piece(hbm, buf, sem, r0, rn, c0, cn):
        sl = (pl.ds(r0, rn), pl.ds(c0, cn))
        return hbm.at[sl], buf.at[sl], sem

    wq_cols = H * DH // WQ_C
    n_wq = (D_MODEL // WQ_R) * wq_cols

    def wq_piece(k):
        n = lax.rem(k * 11, jnp.int32(n_wq))
        r = lax.div(n, jnp.int32(wq_cols))
        c = n - wq_cols * r
        return piece(wq_hbm, wqbuf, wsem.at[0],
                     pl.multiple_of(r * WQ_R, WQ_R), WQ_R, pl.multiple_of(c * WQ_C, 128), WQ_C)

    wo_per_slice = GR // WO_R

    def wo_piece(k):
        k = jnp.asarray(k, jnp.int32)
        gg = lax.div(k, jnp.int32(wo_per_slice))
        n = lax.rem((k - gg * wo_per_slice) * 7, jnp.int32(wo_per_slice))
        return piece(wo_hbm, wobuf, wsem.at[gg], pl.multiple_of(gg * GR + n * WO_R, WO_R), WO_R, 0, D_MODEL)

    def issue_wo(n):
        def f(i, carry):
            k = SKEW + 2 * (n * WO_PER_STEP + i)

            @pl.when(k < GPB * wo_per_slice)
            def _():
                start_pair(wo_piece(k), wo_piece(k + 1))
            return carry
        lax.fori_loop(0, WO_PER_STEP, f, 0, unroll=4)

    def ffn_sem(j):
        return kvsem.at[j // NQ, j % NQ]

    gu_lo = [sum(GU_GROUPS[:i]) for i in range(len(GU_GROUPS))]
    wd_lo = [sum(WD_GROUPS[:i]) for i in range(len(WD_GROUPS))]
    tail = []
    for i, n in enumerate(GU_GROUPS):
        for k in range(n // GU_R):
            tail.append(piece(wg_hbm, wgbuf, ffn_sem(i), gu_lo[i] + k * GU_R, GU_R, 0, FF))
            tail.append(piece(wu_hbm, wubuf, ffn_sem(i), gu_lo[i] + k * GU_R, GU_R, 0, FF))
    for i, n in enumerate(WD_GROUPS):
        for k in _scattered(n // WO_R, 7 if (n // WO_R) % 5 == 0 else 5):
            tail.append(piece(wd_hbm, wdbuf, ffn_sem(len(GU_GROUPS) + i), wd_lo[i] + k * WO_R, WO_R, 0, D_MODEL))
    tail_pos = [0]

    def issue_tail(n):
        lo = tail_pos[0]
        hi = min(lo + 2 * n, len(tail))
        for k in range(lo, hi, 2):
            start_pair(tail[k], tail[k + 1])
        tail_pos[0] = hi

    cx = pltpu.make_async_copy(x_hbm, xbuf, wsem.at[0])
    cwr = pltpu.make_async_copy(wr_hbm, wrbuf, wsem.at[0])

    row8 = lax.broadcasted_iota(jnp.int32, (8, GR), 0)
    lane8 = lax.broadcasted_iota(jnp.int32, (8, GR), 1)
    bd_mask = (lane8 >= row8 * DH) & (lane8 < (row8 + 1) * DH)

    cx.start(priority=TB)
    cwr.start(priority=TA)
    for j in range(SKEW):
        pltpu.make_async_copy(*kv_copy(0, 0, j, 1)).start(priority=TB)

    def first_wq(i, carry):
        start_pair(wq_piece(2 * i), wq_piece(2 * i + 1))
        return carry
    lax.fori_loop(0, n_wq // 2, first_wq, 0, unroll=4)
    issue_kv(0, 0)
    issue_kv(0, 1)
    m_scr[...] = jnp.full(m_scr.shape, -jnp.inf, F32)
    l_scr[...] = jnp.zeros(l_scr.shape, F32)
    o_scr[...] = jnp.zeros(o_scr.shape, F32)
    cx.wait()
    cwr.wait()
    wait((wq_hbm, wqbuf, wsem.at[0]))
    ln1 = _ln(xbuf[...].astype(F32)).astype(BF16)

    def q_proj(gg, carry):
        cols = pl.ds(pl.multiple_of(gg * GR, 128), GR)
        q = jnp.dot(ln1, wqbuf[:, cols], preferred_element_type=F32)
        for b in range(B):
            qb = jnp.broadcast_to(q[b:b + 1, :], (8, GR))
            qbd_scr[b * GPB + gg] = jnp.where(bd_mask, qb, 0.0).astype(BF16)

        @pl.when(jnp.bitwise_and(gg, 1) == 1)
        def _():
            issue_half_pass(2 + lax.shift_right_logical(gg, 1))
        return carry
    lax.fori_loop(0, GPB, q_proj, 0)

    def rest(m, carry):
        issue_half_pass(m)
        return carry
    lax.fori_loop(4, AHEAD, rest, 0)

    def step(c, g):
        slot = lax.rem(c, jnp.int32(NR))
        rows = pl.ds(g * GA, GA)
        s = jnp.dot(qbd_scr[g], kbuf[slot, rows].reshape(GR, CW), preferred_element_type=F32)
        m_old = m_scr[g]
        m_new = jnp.maximum(m_old, jnp.broadcast_to(jnp.max(s, axis=1, keepdims=True), (8, CW)))
        alpha = jnp.exp((m_old - m_new) * SCALE)
        p = jnp.exp((s - m_new) * SCALE)
        m_scr[g] = m_new
        l_scr[g] = l_scr[g] * alpha + p
        pv = lax.dot_general(p.astype(BF16), vbuf[slot, rows].reshape(GR, CW), (((1,), (1,)), ((), ())),
                             preferred_element_type=F32)
        o_scr[g] = o_scr[g] * alpha[:, 0:1] + pv

    def super_step(n, carry):
        c = lax.shift_right_logical(n, 3)
        i = jnp.bitwise_and(n, NSS - 1)

        @pl.when(jnp.bitwise_and(i, NSS // NQ - 1) == 0)
        def _():
            q = lax.div(i, jnp.int32(NSS // NQ))
            wait(kv_part(k_hbm, kbuf, c, q))
            wait(kv_part(v_hbm, vbuf, c, q))
        step(c, 2 * i)
        step(c, 2 * i + 1)

        m = n + AHEAD
        issue_half_pass(m)
        nw = m - NC * NSS

        @pl.when((nw >= 0) & (nw < -(-(GPB * wo_per_slice - SKEW) // (2 * WO_PER_STEP))))
        def _():
            issue_wo(nw)
        return carry

    lax.fori_loop(0, NC * NSS, super_step, 0)

    attn = jnp.zeros((8, D_MODEL), F32)
    for gg in range(GPB):
        issue_tail(TAIL_PER_SLICE[gg])
        oin = jnp.zeros((8, GR), F32)
        for b in range(B):
            g = b * GPB + gg
            l = jnp.sum(l_scr[g], axis=1, keepdims=True)
            o = jnp.where(bd_mask, o_scr[g] / l, 0.0)
            orow = jnp.sum(o, axis=0, keepdims=True)
            oin = jnp.where(row8 == b, jnp.broadcast_to(orow, (8, GR)), oin)
        sl = pl.ds(gg * GR, GR)
        wait((wo_hbm.at[sl], wobuf.at[sl], wsem.at[gg]))
        attn = attn + jnp.dot(oin.astype(BF16), wobuf[sl, :], preferred_element_type=F32)

    h = xbuf[...].astype(F32) + attn[0:B, :]
    ln2 = _ln(h)
    ln2b = ln2.astype(BF16)
    r = jnp.sum(ln2b.astype(F32) * wrbuf[...].astype(F32)[None, :], axis=1, keepdims=True)
    issue_tail(len(tail))
    gt = jnp.zeros((B, FF), F32)
    up = jnp.zeros((B, FF), F32)
    for i, n in enumerate(GU_GROUPS):
        sl = pl.ds(gu_lo[i], n)
        wait((wg_hbm.at[sl], wgbuf.at[sl], ffn_sem(i)))
        wait((wu_hbm.at[sl], wubuf.at[sl], ffn_sem(i)))
        lhs = ln2b[:, gu_lo[i]:gu_lo[i] + n]
        gt = gt + jnp.dot(lhs, wgbuf[sl, :], preferred_element_type=F32)
        up = up + jnp.dot(lhs, wubuf[sl, :], preferred_element_type=F32)
    act = (gt * jax.nn.sigmoid(gt) * up).astype(BF16)
    y = jnp.zeros((B, D_MODEL), F32)
    for i, n in enumerate(WD_GROUPS):
        sl = pl.ds(wd_lo[i], n)
        wait((wd_hbm.at[sl], wdbuf.at[sl], ffn_sem(len(GU_GROUPS) + i)))
        y = y + jnp.dot(act[:, wd_lo[i]:wd_lo[i] + n], wdbuf[sl, :], preferred_element_type=F32)
    out = h + (ln2 + y * jax.nn.sigmoid(r))
    out_ref[...] = out.astype(out_ref.dtype)


@jax.jit
def pallas_sequential_preLN__mha_block_cached__moe_arch_mod__decode_kernel(
    A_x, A_k_cache, A_v_cache, A_wq, A_wo, B_x, B_w_r, B_w_gate, B_w_up, B_w_down
):
    del B_x
    kt = jnp.swapaxes(A_k_cache, 2, 3).reshape(NA, 2, 8, SK)
    vt = jnp.swapaxes(A_v_cache, 2, 3).reshape(NA, 2, 8, SK)
    x2 = A_x.reshape(B, D_MODEL)
    anyspec = pl.BlockSpec(memory_space=pl.ANY)
    ring = pltpu.VMEM((NR, NA, 2, 8, CW), BF16)
    out = pl.pallas_call(
        _kernel,
        in_specs=[anyspec] * 9,
        out_specs=pl.BlockSpec(memory_space=pltpu.VMEM),
        out_shape=jax.ShapeDtypeStruct((B, D_MODEL), BF16),
        scratch_shapes=[
            pltpu.VMEM((B, D_MODEL), BF16),
            pltpu.VMEM((D_MODEL,), BF16),
            pltpu.VMEM((D_MODEL, H * DH), BF16),
            pltpu.VMEM((H * DH, D_MODEL), BF16),
            pltpu.VMEM((D_MODEL, FF), BF16),
            pltpu.VMEM((D_MODEL, FF), BF16),
            pltpu.VMEM((FF, D_MODEL), BF16),
            ring, ring,
            pltpu.VMEM((NG, 8, GR), BF16),
            pltpu.VMEM((NG, 8, CW), F32),
            pltpu.VMEM((NG, 8, CW), F32),
            pltpu.VMEM((NG, 8, GR), F32),
            pltpu.SemaphoreType.DMA((NR, NQ)),
            pltpu.SemaphoreType.DMA((GPB,)),
        ],
        compiler_params=pltpu.CompilerParams(vmem_limit_bytes=100 * 1024 * 1024),
    )(x2, kt, vt, A_wq, A_wo, B_w_r, B_w_gate, B_w_up, B_w_down)
    return out.reshape(B, 1, D_MODEL)
```
